```python
import os as _os
_os.environ.setdefault("JAX_PLATFORMS", "cpu")
import jax
import jax.numpy as jnp

def _softmax(x, axis=-1):
    return jax.nn.softmax(x, axis=axis)
def _gelu(x):
    return jax.nn.gelu(x, approximate=True)
def _silu(x):
    return jax.nn.silu(x)
def _sigmoid(x):
    return jax.nn.sigmoid(x)
def _layernorm(x, axis=-1, eps=1e-5):
    m = jnp.mean(x, axis=axis, keepdims=True)
    v = jnp.var(x, axis=axis, keepdims=True)
    return (x - m) / jnp.sqrt(v + eps)
def _scatter_add(tgt, idx, src, axis=0):
    return tgt.at[idx].add(src)
def _segment_sum(src, seg, n):
    return jax.ops.segment_sum(src, seg, n)
class _Rng:
    def __init__(self, key):
        self._k = key
    def _next(self):
        self._k, sub = jax.random.split(self._k)
        return sub
    def normal(self, shape):
        return jax.random.normal(self._next(), shape, dtype=jnp.bfloat16)
    def randint(self, lo, hi, shape):
        return jax.random.randint(self._next(), shape, lo, hi, dtype=jnp.int32)
    def uniform(self, shape, lo=0.0, hi=1.0):
        return jax.random.uniform(self._next(), shape, jnp.bfloat16, lo, hi)
    def permutation(self, n):
        return jax.random.permutation(self._next(), n)


kernel_name = 'sequential_preLN__sliding_block__dense_activation_gelu__prompt'

def setup_inputs():
    _rng = _Rng(jax.random.key(int.from_bytes(__import__("os").urandom(4), "little")))
    _w = (lambda a: (lambda t: t.astype(jnp.bfloat16) if jnp.issubdtype(t.dtype, jnp.floating) else t)(jnp.asarray(a)))
    def _A_setup():
        B, S, D = 1, 2048, 640
        return {
            "x": _w((lambda *s: _rng.normal(s) * 0.05)(B, S, D)),
            "wqkv": _w((lambda *s: _rng.normal(s) * 0.05)(D, 3 * D)),
            "wo": _w((lambda *s: _rng.normal(s) * 0.05)(D, D)),
        }
    _A_in = _A_setup()

    def _B_setup():
        B, S, D, F = 1, 2048, 640, 1536
        return {
            "x": _w((lambda *s: _rng.normal(s) * 0.05)(B, S, D)),
            "w1": _w((lambda *s: _rng.normal(s) * 0.8)(D, F) * (D ** -0.5)),
            "b1": _w((lambda *s: _rng.normal(s) * 0.8)(F) * 0.01),
            "w2": _w((lambda *s: _rng.normal(s) * 0.8)(F, D) * (F ** -0.5)),
            "b2": _w((lambda *s: _rng.normal(s) * 0.05)(D) * 0.01),
        }
    _B_in = _B_setup()

    return {
        "A_x": _A_in["x"],
        "A_wqkv": _A_in["wqkv"],
        "A_wo": _A_in["wo"],
        "B_x": _B_in["x"],
        "B_w1": _B_in["w1"],
        "B_b1": _B_in["b1"],
        "B_w2": _B_in["w2"],
        "B_b2": _B_in["b2"],
    }

def reference(A_x, A_wqkv, A_wo, B_x, B_w1, B_b1, B_w2, B_b2):
    def _A_ref(x, wqkv, wo):
        B, S, D = x.shape
        H = 32; Dh = D // H; W = 256
        qkv = (lambda x, *d: x.transpose(*d))((x @ wqkv).reshape(B, S, 3, H, Dh), 2, 0, 3, 1, 4)
        q, k, v = qkv[0], qkv[1], qkv[2]
        scores = jnp.einsum("bhqd,bhkd->bhqk", q, k) * (Dh ** -0.5)
        idx = jnp.arange(S)
        mask = (idx[:, None] - idx[None, :] >= 0) & (idx[:, None] - idx[None, :] < W)
        scores = jnp.where(mask[None, None], scores, -1e9)
        p = _softmax(scores, axis=-1)
        o = jnp.einsum("bhqk,bhkd->bhqd", p, v)
        return (lambda x, *d: x.transpose(*d))(o, 0, 2, 1, 3).reshape(B, S, D) @ wo

    def _B_ref(x, w1, b1, w2, b2):
        h = jnp.einsum("bsd,df->bsf", x, w1) + b1
        h = _gelu(h)
        return jnp.einsum("bsf,fd->bsd", h, w2) + b2

    x = A_x
    h = x + _A_ref(_layernorm(x, axis=-1), A_wqkv, A_wo)
    h2 = h + _B_ref(_layernorm(h, axis=-1), B_w1, B_b1, B_w2, B_b2)
    return h2
```

```python
import functools
import numpy as np
import jax
import jax.numpy as jnp
import jax.experimental.pallas as pl
import jax.experimental.pallas.tpu as pltpu

S, D, F, H, W = 2048, 640, 1536, 32, 256
DH = D // H
NG = 8
GF = 4 * DH
TB = 256
NEG = -1e9
LOG2E = 1.4426950408889634
bf16, f32, i32 = jnp.bfloat16, jnp.float32, jnp.int32
NT = (((1,), (1,)), ((), ()))


def _ln(x):
    m = jnp.mean(x, axis=-1, keepdims=True)
    xc = x - m
    v = jnp.mean(xc * xc, axis=-1, keepdims=True)
    return xc * jax.lax.rsqrt(v + 1e-5)


def _slabs(y):
    lo = jax.lax.broadcasted_iota(i32, (y.shape[0], 128), 1) < 64
    s = [y[:, 128 * j:128 * (j + 1)] for j in range(5)]
    m = lambda a: jnp.where(lo, s[a + 1], s[a])
    return [s[0], m(0), s[1], m(1), m(2), s[3], m(3), s[4]]


def _kernel(x_ref, wqkv_h, wo_h, w1_h, b1_ref, w2_h, b2_ref, o_ref,
            wqkv, wo, w1, w2, q_s, k_s, vt_s, ot_s, sem, tri_s, f0, f1, p0, p1, *, NC, ER):
    f_s, p_s = (f0, f1), (p0, p1)
    i = pl.program_id(0)
    cps = [pltpu.make_async_copy(s, d, sem.at[n]) for n, (s, d) in
           enumerate([(wqkv_h, wqkv), (wo_h, wo), (w1_h, w1), (w2_h, w2)])]

    @pl.when(i == 0)
    def _():
        for c in cps:
            c.start()

    x = x_ref[...].astype(f32)
    xn = _ln(x).astype(bf16)

    @pl.when(i == 0)
    def _():
        cps[0].wait()

    t0 = pl.multiple_of(i * TB, TB)
    q = jnp.dot(xn, wqkv[:, 0:D], preferred_element_type=f32) * (DH ** -0.5 * LOG2E)
    for g, s in enumerate(_slabs(q)):
        q_s[g] = s.astype(bf16)
    k = jnp.dot(xn, wqkv[:, D:2 * D], preferred_element_type=f32)
    for g, s in enumerate(_slabs(k)):
        k_s[g, pl.ds(t0, TB), :] = s.astype(bf16)
    v = jnp.dot(xn, wqkv[:, 2 * D:3 * D], preferred_element_type=f32)
    vt = v.T.astype(bf16)
    for b in range(TB // 128):
        vt_s[i * (TB // 128) + b] = vt[:, 128 * b:128 * (b + 1)]

    row = jax.lax.broadcasted_iota(i32, (128, 128), 0)
    col = jax.lax.broadcasted_iota(i32, (128, 128), 1)

    @pl.when(i == 0)
    def _():
        for hh in range(4):
            t = pltpu.bitcast(jnp.where(row > ((col + 32 * hh) & 127), 1.0, 0.0).astype(bf16), i32)
            t = (t >> 7) & 0x00010001
            tri_s[hh] = (t << 16) - t

    lane = jax.lax.broadcasted_iota(i32, (8, 128), 1)
    tri32 = row[:32] > (col[:32] & 31)
    negc = NEG * LOG2E

    def merge(p):
        c = jax.lax.broadcasted_iota(i32, p[0].shape, 1)
        i0, i1 = (c & 32) != 0, (c & 64) != 0
        u = [jnp.where(i0, p[(a + 1) % 4], p[a]) for a in range(4)]
        return [jnp.where(i1, u[(a + 2) % 4], u[a]) for a in range(4)]

    class Unit:
        def __init__(self, n, g, b, nprev):
            self.g, self.b, self.nprev, self.sl = g, b, nprev, n % 2
            self.mx, self.l = [None] * 4, [None] * 4
            self.blk = i * (TB // 128) + b

        def qk(self, j):
            g, b, nprev = self.g, self.b, self.nprev
            qb = pltpu.bitcast(q_s[g, 128 * b + 32 * j:128 * b + 32 * j + 32, :], i32).reshape(2, 8, 128)
            parts = []
            for ii in range(4):
                h = 4 * g + (j - ii) % 4
                lm = jnp.where(((lane - DH * h) & 127) < DH, -1, 0)
                parts.append((qb & lm[None]).reshape(16, 128))
            qm = pltpu.bitcast(jnp.concatenate(parts, axis=0), bf16)
            ts = max(0, 256 - 128 * nprev - 32 * j)
            k0 = pl.multiple_of(self.blk * 128 - 256 + 32 * j + ts, 32)
            s = jax.lax.dot_general(k_s[g, pl.ds(k0, 288 - ts), :], qm, NT, preferred_element_type=f32)
            fs = f_s[self.sl]
            d = jnp.where(tri32, s[:32] if ts == 0 else negc, s[256 - ts:])
            fs[j, 32 * j:32 * j + 32] = d
            mx = d
            for t in range(32, 256, 32):
                r = (32 * j + t) % 256
                if t >= ts:
                    v = s[t - ts:t - ts + 32]
                    mx = jnp.maximum(mx, v)
                    fs[j, r:r + 32] = v
                elif r < 128:
                    fs[j, r:r + 32] = jnp.full((32, 128), negc, f32)
            self.mx[j] = jnp.max(mx, axis=0, keepdims=True)

        def ex(self, c, nc):
            rows = (256 if self.nprev else 128) // nc
            for r in range(c * rows, (c + 1) * rows, ER):
                p = []
                for j in range(4):
                    e = jnp.exp2(f_s[self.sl][j, r:r + ER] - self.mx[j])
                    es = e.reshape(ER // 8, 8, 128).sum(axis=0)
                    self.l[j] = es if self.l[j] is None else self.l[j] + es
                    p.append(pltpu.bitcast(e.astype(bf16), i32))
                for hh, v in enumerate(merge(p)):
                    p_s[self.sl][hh, r // 2:(r + ER) // 2] = v
            if c == nc - 1:
                self.rl = merge([1.0 / jnp.sum(l, axis=0, keepdims=True) for l in self.l])
                self.parts = []

        def pv(self, hh):
            g, blk = self.g, self.blk
            pf = p_s[self.sl][hh, 0:64]
            r0 = (DH * hh) // 16 * 16
            off = DH * hh - r0
            rr = slice(g * GF + r0, g * GF + r0 + 32)
            if self.nprev == 2:
                pa = pf & tri_s[hh]
                pf = pf ^ pa
            o = jnp.dot(vt_s[blk, rr, :], pltpu.bitcast(pf, bf16), preferred_element_type=f32)
            if self.nprev >= 1:
                o += jnp.dot(vt_s[blk - 1, rr, :], pltpu.bitcast(p_s[self.sl][hh, 64:128], bf16), preferred_element_type=f32)
            if self.nprev == 2:
                o += jnp.dot(vt_s[blk - 2, rr, :], pltpu.bitcast(pa, bf16), preferred_element_type=f32)
            o8 = off // 8 * 8
            o = o[o8:o8 + 24] * self.rl[hh]
            if hh:
                o = pltpu.roll(o, 32 * hh, 1)
            self.parts.append(o[off - o8:off - o8 + DH])
            if hh == 3:
                ot_s[g * GF:(g + 1) * GF, 128 * self.b:128 * self.b + 128] = jnp.concatenate(self.parts, axis=0)

    def attention(first):
        us = [(g, b) for b in range(TB // 128) for g in range(NG)]
        us = [Unit(n, g, b, min(b, 2) if first else 2) for n, (g, b) in enumerate(us)]
        n = len(us)
        for t in range(n + 2):
            for c in range(NC):
                for j in range(c * 4 // NC, (c + 1) * 4 // NC):
                    if t < n:
                        us[t].qk(j)
                if 0 <= t - 1 < n:
                    us[t - 1].ex(c, NC)
                for j in range(c * 4 // NC, (c + 1) * 4 // NC):
                    if 0 <= t - 2 < n:
                        us[t - 2].pv(j)

    @pl.when(i == 0)
    def _():
        attention(True)
        for c in cps[1:]:
            c.wait()

    @pl.when(i > 0)
    def _():
        attention(False)

    o = ot_s[...].T.astype(bf16)
    h = x_ref[...].astype(f32) + jnp.dot(o, wo[...], preferred_element_type=f32)
    hn = _ln(h).astype(bf16)
    u = jnp.dot(hn, w1[...], preferred_element_type=f32) + b1_ref[...].astype(f32)
    u = jax.nn.gelu(u, approximate=True).astype(bf16)
    y = jnp.dot(u, w2[...], preferred_element_type=f32) + b2_ref[...].astype(f32)
    o_ref[...] = (h + y).astype(o_ref.dtype)


def run(A_x, A_wqkv, A_wo, B_x, B_w1, B_b1, B_w2, B_b2, NC=4, ER=16):
    del B_x
    hbm = pl.BlockSpec(memory_space=pl.ANY)
    out = pl.pallas_call(
        functools.partial(_kernel, NC=NC, ER=ER),
        grid=(S // TB,),
        in_specs=[pl.BlockSpec((None, TB, D), lambda i: (0, i, 0)), hbm, hbm, hbm,
                  pl.BlockSpec((1, F), lambda i: (0, 0)), hbm,
                  pl.BlockSpec((1, D), lambda i: (0, 0))],
        out_specs=pl.BlockSpec((None, TB, D), lambda i: (0, i, 0)),
        out_shape=jax.ShapeDtypeStruct((1, S, D), bf16),
        scratch_shapes=[pltpu.VMEM((D, 3 * D), bf16), pltpu.VMEM((D, D), bf16),
                        pltpu.VMEM((D, F), bf16), pltpu.VMEM((F, D), bf16),
                        pltpu.VMEM((NG, TB, 128), bf16), pltpu.VMEM((NG, S, 128), bf16),
                        pltpu.VMEM((S // 128, D, 128), bf16), pltpu.VMEM((D, TB), f32),
                        pltpu.SemaphoreType.DMA((4,)), pltpu.VMEM((4, 64, 128), i32),
                        *[pltpu.VMEM((4, 256, 128), f32)] * 2, *[pltpu.VMEM((4, 128, 128), i32)] * 2],
        compiler_params=pltpu.CompilerParams(dimension_semantics=("arbitrary",),
                                             vmem_limit_bytes=100 * 1024 * 1024),
    )(A_x, A_wqkv, A_wo, B_w1, B_b1.reshape(1, F), B_w2, B_b2.reshape(1, D))
    return out


@jax.jit
def pallas_sequential_preLN__sliding_block__dense_activation_gelu__prompt_kernel(
        A_x, A_wqkv, A_wo, B_x, B_w1, B_b1, B_w2, B_b2):
    return run(A_x, A_wqkv, A_wo, B_x, B_w1, B_b1, B_w2, B_b2)
```

```python
import functools
import numpy as np
import jax
import jax.numpy as jnp
import jax.experimental.pallas as pl
import jax.experimental.pallas.tpu as pltpu

S, D, F, H, W = 2048, 640, 1536, 32, 256
DH = D // H
NG = 8
TB = 256
NB = TB // 128
NT_ = S // TB
NEG = -1e9
LOG2E = 1.4426950408889634
bf16, f32, i32 = jnp.bfloat16, jnp.float32, jnp.int32
NT = (((1,), (1,)), ((), ()))
HI = -65536
dot = functools.partial(jnp.dot, preferred_element_type=f32)


def _ln(x):
    m = jnp.mean(x, axis=-1, keepdims=True)
    xc = x - m
    v = jnp.mean(xc * xc, axis=-1, keepdims=True)
    return xc * jax.lax.rsqrt(v + 1e-5)


def _ilv(y, rnd):
    n, c = y.shape
    b = pltpu.bitcast(y, i32)
    if rnd:
        b = b + 0x8000
    b = b.reshape(n // 16, 2, 8, c)
    w = jax.lax.shift_right_logical(b[:, 0], 16) | (b[:, 1] & HI)
    return w.reshape(n // 2, c)


def _kernel(x_h, wqkv_h, wo_h, w1_h, b1_ref, w2_h, b2_ref, o_ref,
            x_s, wqkv, wo, w1, w2, q_s, k_s, vt_s, o_s, sem, tri_s, xn_s, f0, f1, p0, p1, *, P):
    i = pl.program_id(0)
    zs, zl = (i // 1024, i // 2048) if P["OPQ"] else (0, 0)
    never = jax.lax.broadcasted_iota(i32, (8, 128), 1) < i // 4096
    pairs = [(x_h.at[0, 0:2 * TB], x_s.at[0:2 * TB])]
    pairs += [(wqkv_h.at[:, c:c + D], wqkv.at[:, c:c + D]) for c in range(0, 3 * D, D)]
    pairs += [(wo_h, wo), (x_h.at[0, 2 * TB:S], x_s.at[2 * TB:S]), (w1_h, w1), (w2_h, w2)]
    cps = [pltpu.make_async_copy(s, d, sem.at[n]) for n, (s, d) in enumerate(pairs)]

    def rows(t):
        return pl.ds(pl.multiple_of(t * TB, TB), TB)

    def lin(a, w, c0, n, fin):
        items, st = [], {}
        kk = w.shape[0]
        for c in range(0, n, 512):
            e = min(c + 512, n)
            if kk % 512:
                def rem(c=c, e=e):
                    st[c] = dot(a()[:, 512:], w[512:, c0 + c:c0 + e])
                    return st[c]
                items.append(((e - c) // 2, rem))
            for cc in range(c, e, 128):
                for k in range(0, kk - 511, 512):
                    def main(c=c, cc=cc, k=k):
                        y = dot(a()[:, k:k + 512], w[k:k + 512, c0 + cc:c0 + cc + 128])
                        if k:
                            y = y + st["acc"]
                        elif kk % 512:
                            y = y + st[c][:, cc - c:cc - c + 128]
                        st["acc"] = y
                        if k + 1024 > kk:
                            fin(cc, y)
                        return y
                    items.append((256, main))
        return items

    def qkv_items(t, pre=None):
        st = {} if pre is None else {"xn": pre}

        def xn():
            if "xn" not in st:
                st["xn"] = _ln(x_s[rows(t), :].astype(f32)).astype(bf16)
            return st["xn"]
        lo = jax.lax.broadcasted_iota(i32, (TB // 2, 128), 1) < 64
        hrows = pl.ds(pl.multiple_of(t * (TB // 2), TB // 2), TB // 2)

        def slab(dst, scale):
            def fin(c, y):
                j = c // 128
                y = pltpu.bitcast((y * scale if scale else y).astype(bf16), i32)
                if j != 2:
                    later.append(lambda: dst.__setitem__(((0, 2, None, 5, 7)[j], hrows), y))
                if j:
                    m = jnp.where(lo, y, st["prev"])
                    later.append(lambda: dst.__setitem__(((None, 1, 3, 4, 6)[j], hrows), m))
                st["prev"] = y
            return fin

        def vfin(c, y):
            st[c] = pltpu.bitcast(pltpu.bitcast(_ilv(y, True), bf16).T, i32)
            sub = jax.lax.broadcasted_iota(i32, (8, TB), 0)
            for h in range(H):
                r0 = DH * h // 16 * 8
                if (r0 + 8) // 64 != c // 128:
                    continue
                a, b = (st[r // 64 * 128][r % 64:r % 64 + 8] for r in (r0, r0 + 8))
                if h % 4 < 2:
                    b = jnp.where(sub >= 4, 0x3F803F80, b)
                else:
                    a = jnp.where(sub < 4, 0x3F803F80, a)
                w = jnp.concatenate([a, b], axis=0)
                for bb in range(NB):
                    later.append(lambda w=w, h=h, bb=bb: vt_s.__setitem__((t * NB + bb, h), w[:, 128 * bb:128 * (bb + 1)]))
        fins = (slab(q_s, DH ** -0.5 * LOG2E), slab(k_s, None), vfin)
        return [lin(xn, wqkv, D * n, D, fins[n]) for n in range(3)]

    def mlp_items():
        hs, us, st = [], [], {}

        def once(key, fn):
            if key not in st:
                st[key] = fn()
            return st[key]

        def f_o(c, y):
            hs.append(x_s[rows(i - 1), c:c + 128].astype(f32) + y)

        def f_up(c, y):
            u = y + b1_ref[c:c + 128].astype(f32).reshape(1, 128)
            us.append(jax.nn.gelu(u, approximate=True).astype(bf16))

        def f_dn(c, y):
            y = y + b2_ref[c:c + 128].astype(f32).reshape(1, 128)
            o_ref[:, c:c + 128] = (hs[c // 128] + y).astype(o_ref.dtype)
        o = pltpu.bitcast(o_s[...], bf16)
        hn = lambda: once("hn", lambda: _ln(jnp.concatenate(hs, axis=1)).astype(bf16))
        u = lambda: once("u", lambda: jnp.concatenate(us, axis=1))
        return lin(lambda: o, wo, 0, D, f_o), lin(hn, w1, 0, F, f_up) + lin(u, w2, 0, D, f_dn)

    lane = jax.lax.broadcasted_iota(i32, (8, 128), 1)
    tri32 = jax.lax.broadcasted_iota(i32, (32, 128), 0) > (jax.lax.broadcasted_iota(i32, (32, 128), 1) & 31)
    negc = NEG * LOG2E
    later = []

    def flush():
        for fn in later:
            fn()
        later.clear()

    def merge(p):
        c = jax.lax.broadcasted_iota(i32, p[0].shape, 1)
        i0, i1 = (c & 32) != 0, (c & 64) != 0
        u = [jnp.where(i0, p[(a + 1) % 4], p[a]) for a in range(4)]
        return [jnp.where(i1, u[(a + 2) % 4], u[a]) for a in range(4)]

    class Unit:
        def __init__(self, n, g, b, nprev, ot):
            self.g, self.b, self.nprev, self.ot = g, b, nprev, ot
            self.f, self.p = (f0, f1)[n % 2], (p0, p1)[n % 2]
            self.mx, self.blk = [None] * 4, i * NB + b

        def qk(self, j):
            g, nprev = self.g, self.nprev
            qb = q_s[g, pl.ds(pl.multiple_of(self.blk * 64 + 16 * j, 16), 16), :].reshape(2, 8, 128)
            parts = []
            for ii in range(4):
                h = 4 * g + (j - ii) % 4
                lm = jnp.where(((lane - DH * h) & 127) < DH, -1, 0)
                parts.append((qb & lm[None]).reshape(16, 128))
            qm = pltpu.bitcast(jnp.concatenate(parts, axis=0), bf16)
            ts = max(0, 256 - 128 * nprev - 32 * j)
            k0 = pl.multiple_of(self.blk * 64 - 128 + 16 * j + ts // 2, 16)
            kk = pltpu.bitcast(k_s[g, pl.ds(k0, 144 - ts // 2), :], bf16)
            s = jax.lax.dot_general(kk, qm, NT, preferred_element_type=f32)
            d = jnp.where(tri32, s[:32] if ts == 0 else negc, s[256 - ts:])
            self.f[zs, j, 32 * j:32 * j + 32] = d
            mx = d
            for t in range(32, 256, 32):
                r = (32 * j + t) % 256
                if t >= ts:
                    v = s[t - ts:t - ts + 32]
                    mx = jnp.maximum(mx, v)
                    self.f[zs, j, r:r + 32] = v
                elif r < 128:
                    self.f[zs, j, r:r + 32] = jnp.full((32, 128), negc, f32)
            self.mx[j] = jnp.broadcast_to(jnp.max(mx, axis=0, keepdims=True), (8, 128))

        def ex(self, c, nc, tick):
            n = (256 if self.nprev else 128) // nc
            mx = [m if tick is None else jnp.where(never, tick, m) for m in self.mx]
            for r in range(c * n, (c + 1) * n, 16):
                p = [_ilv(jnp.exp2((self.f[zl, j, r:r + 16].reshape(2, 8, 128) - mx[j][None]).reshape(16, 128)), False)
                     for j in range(4)]
                for hh, v in enumerate(merge(p)):
                    self.p[zs, hh, r // 2:r // 2 + 8] = v

        def pv(self, hh):
            g, blk = self.g, self.blk
            h = 4 * g + hh
            mm = lambda bk, p: dot(pltpu.bitcast(vt_s[bk, h], bf16), pltpu.bitcast(p, bf16))
            pf = self.p[zl, hh, 0:64]
            if self.nprev == 2:
                pa = pf & tri_s[hh]
                pf = pf ^ pa
            o = mm(blk, pf)
            if self.nprev >= 1:
                o += mm(blk - 1, self.p[zl, hh, 64:128])
            if self.nprev == 2:
                o += mm(blk - 2, pa)
            l, o = (o[24:], o[:24]) if hh < 2 else (o[:8], o[8:])
            o = (o.reshape(3, 8, 128) * (1.0 / l)[None]).reshape(24, 128)
            if hh:
                o = pltpu.roll(o, 32 * hh, 1)
            off = 4 * (hh % 2)
            self.ot.append(o[off:off + DH])
            if h == H - 1:
                o_s[64 * self.b:64 * self.b + 64] = pltpu.bitcast(jnp.concatenate(self.ot, axis=0).T.astype(bf16), i32)

    def attend(first, dense, a0, a1):
        ots = [[] for _ in range(NB)]
        us = [(g, b) for b in range(NB) for g in range(NG)]
        us = [Unit(n, g, b, min(b, 2) if first else 2, ots[b]) for n, (g, b) in enumerate(us)]
        n, nc = len(us), (8 if first else P["NC"])
        tot, done = sum(w for w, _ in dense), 0

        def run(upto):
            nonlocal done
            out = []
            while dense and done + dense[0][0] // 2 <= upto:
                w, it = dense.pop(0)
                done += w
                out.append(it())
            return out
        run(a0)
        for t in range(n + 2):
            if t < n:
                for j in range(4):
                    us[t].qk(j)
            flush()
            if t >= 2:
                for j in range(4):
                    us[t - 2].pv(j)
            ys = run(a0 + (tot - a0 - a1) * t // n if t <= n else tot)
            if 1 <= t <= n:
                for c in range(nc):
                    tick = None
                    if ys and P["TIE"]:
                        pos = int(c * len(ys) * TB * P["TIE"]) // nc // 8 * 8
                        tick = ys[pos // TB][pos % TB:pos % TB + 8, :128]
                    us[t - 1].ex(c, nc, tick)
        flush()

    @pl.when(i == 0)
    def _():
        cps[0].start(), cps[1].start()
        row = jax.lax.broadcasted_iota(i32, (128, 128), 0)
        col = jax.lax.broadcasted_iota(i32, (128, 128), 1)
        for hh in range(4):
            tri_s[hh] = _ilv(pltpu.bitcast(jnp.where(row > ((col + 32 * hh) & 127), -1, 0), f32), False)
        cps[0].wait()
        cps[2].start()
        xn_s[...] = pltpu.bitcast(_ln(x_s[0:2 * TB, :].astype(f32)).astype(bf16), i32)
        cps[1].wait()
        cps[3].start()
        a, b = (qkv_items(t, pltpu.bitcast(xn_s[t * TB // 2:(t + 1) * TB // 2], bf16)) for t in range(2))
        for n in range(3):
            if n == 1:
                for c in cps[4:]:
                    c.start()
            if n:
                cps[n + 1].wait()
            for _, it in a[n] + (b[n] if n < P["F0"] else []):
                it()
            flush()
        attend(True, sum(b[P["F0"]:], []), 0, 0)

    @pl.when(i == 1)
    def _():
        for c in cps[4:]:
            c.wait()

    @pl.when((i > 0) & (i < NT_ - 1))
    def _():
        m0, m1 = mlp_items()
        attend(False, m0 + sum(qkv_items(i + 1), []) + m1, P["A0"], P["A1"])

    @pl.when(i == NT_ - 1)
    def _():
        m0, m1 = mlp_items()
        attend(False, m0 + m1, P["B0"], P["B1"])

    @pl.when(i == NT_)
    def _():
        m0, m1 = mlp_items()
        for _, it in m0 + m1:
            it()


def run(A_x, A_wqkv, A_wo, B_x, B_w1, B_b1, B_w2, B_b2, **kw):
    P = dict(NC=8, OPQ=1, TIE=0.65, A0=512, A1=512, B0=1600, B1=1024, F0=2)
    P.update(kw)
    del B_x
    hbm = pl.BlockSpec(memory_space=pl.ANY)
    out = pl.pallas_call(
        functools.partial(_kernel, P=P),
        grid=(NT_ + 1,),
        in_specs=[hbm, hbm, hbm, hbm, pl.BlockSpec((F,), lambda i: (0,)), hbm,
                  pl.BlockSpec((D,), lambda i: (0,))],
        out_specs=pl.BlockSpec((None, TB, D), lambda i: (0, jnp.maximum(i - 1, 0), 0)),
        out_shape=jax.ShapeDtypeStruct((1, S, D), bf16),
        scratch_shapes=[pltpu.VMEM((S, D), bf16), pltpu.VMEM((D, 3 * D), bf16), pltpu.VMEM((D, D), bf16),
                        pltpu.VMEM((D, F), bf16), pltpu.VMEM((F, D), bf16),
                        pltpu.VMEM((NG, S // 2, 128), i32), pltpu.VMEM((NG, S // 2, 128), i32),
                        pltpu.VMEM((S // 128, H, 16, 128), i32), pltpu.VMEM((TB // 2, D), i32),
                        pltpu.SemaphoreType.DMA((8,)), pltpu.VMEM((4, 64, 128), i32), pltpu.VMEM((TB, D), i32),
                        *[pltpu.VMEM((1, 4, 256, 128), f32)] * 2, *[pltpu.VMEM((1, 4, 128, 128), i32)] * 2],
        compiler_params=pltpu.CompilerParams(dimension_semantics=("arbitrary",),
                                             vmem_limit_bytes=100 * 1024 * 1024),
    )(A_x, A_wqkv, A_wo, B_w1, B_b1, B_w2, B_b2)
    return out


@jax.jit
def pallas_sequential_preLN__sliding_block__dense_activation_gelu__prompt_kernel(
        A_x, A_wqkv, A_wo, B_x, B_w1, B_b1, B_w2, B_b2):
    return run(A_x, A_wqkv, A_wo, B_x, B_w1, B_b1, B_w2, B_b2)
```

```python
import functools
import numpy as np
import jax
import jax.numpy as jnp
import jax.experimental.pallas as pl
import jax.experimental.pallas.tpu as pltpu

S, D, F, H, W = 2048, 640, 1536, 32, 256
DH = D // H
NG = 8
TB = 256
NB = TB // 128
NT_ = S // TB
NEG = -1e9
LOG2E = 1.4426950408889634
bf16, f32, i32 = jnp.bfloat16, jnp.float32, jnp.int32
NT = (((1,), (1,)), ((), ()))
HI = -65536
dot = functools.partial(jnp.dot, preferred_element_type=f32)


def _ln(x, gate=None):
    m = jnp.mean(x, axis=-1, keepdims=True)
    if gate:
        m = gate(m)
    xc = x - m
    v = jnp.mean(xc * xc, axis=-1, keepdims=True)
    return xc * jax.lax.rsqrt(v + 1e-5)


def _ilv(y, rnd):
    n, c = y.shape
    b = pltpu.bitcast(y, i32)
    if rnd:
        b = b + 0x8000
    b = b.reshape(n // 16, 2, 8, c)
    w = jax.lax.shift_right_logical(b[:, 0], 16) | (b[:, 1] & HI)
    return w.reshape(n // 2, c)


def mix(a, b):
    return [it for _, it in sorted([(n / len(a), x) for n, x in enumerate(a)] + [(n / (len(b) + 1), x) for n, x in enumerate(b)],
                                   key=lambda q: q[0])]


def _kernel(x_h, wqkv_h, wo_h, w1_h, b1_h, w2_h, b2_h, o_ref, b1_ref, b2_ref,
            x_s, wqkv, wo, w1, w2, q_s, k_s, vt_s, o_s, sem, tri_s, xn_s, xs_s, tq, t1, t2, f0, f1, p0, p1, *, P):
    i = pl.program_id(0)
    never = jax.lax.broadcasted_iota(i32, (8, 128), 1) < i // 4096
    QA = P["QA"]
    pairs = [(x_h.at[0, 0:2 * TB], x_s.at[0:2 * TB])]
    pairs += [(wqkv_h.at[:, c:e], wqkv.at[:, c:e]) for c, e in ((0, QA), (QA, D), (D, 2 * D), (2 * D, 3 * D))]
    pairs += [(x_h.at[0, 2 * TB:4 * TB], x_s.at[2 * TB:4 * TB]), (w1_h, w1), (w2_h, w2),
              (wo_h, wo), (b1_h, b1_ref), (b2_h, b2_ref), (x_h.at[0, 4 * TB:S], x_s.at[4 * TB:S])]
    cps = [pltpu.make_async_copy(s, d, sem.at[n]) for n, (s, d) in enumerate(pairs)]

    def rows(t):
        return pl.ds(pl.multiple_of(t * TB, TB), TB)

    def lin(a, w, c0, n, fin, first=512):
        items, st = [], {}
        kk = w.shape[0]
        cuts = [0] + list(range(first, n, 512)) + [n]
        for c, e in zip(cuts, cuts[1:]):
            if kk % 512:
                def rem(c=c, e=e):
                    st[c] = dot(a()[:, 512:], w[512:, c0 + c:c0 + e])
                    return st[c]
                items.append(((e - c) // 2, rem))
            for cc in range(c, e, 128):
                for k in range(0, kk - 511, 512):
                    def main(c=c, cc=cc, k=k):
                        y = dot(a()[:, k:k + 512], w[k:k + 512, c0 + cc:c0 + cc + 128])
                        if k:
                            y = y + st["acc"]
                        elif kk % 512:
                            y = y + st[c][:, cc - c:cc - c + 128]
                        st["acc"] = y
                        if k + 1024 > kk:
                            later.append(lambda: fin(c0 + cc, y)) if defer else fin(c0 + cc, y)
                        return y
                    items.append((256, main))
        return items

    def prep(w, t, tc, c0, c1):
        kh, items = t.shape[1], []
        for k in range(0, kh, 128):
            def it(k=k):
                b11, b12, b21, b22 = (w[r:r + 128, c:c + 128].astype(f32) for r in (k, k + kh) for c in (c0, c1))
                if seen:
                    y = seen[-1]
                    r = cnt.setdefault(id(y), 0) * 64 % y.shape[0]
                    cnt[id(y)] += 1
                    b12 = jnp.where(never[None], y[r:r + 8, :128][None], b12.reshape(16, 8, 128)).reshape(128, 128)
                u1 = b12 - b11
                u2 = b22 - u1
                for n, v in enumerate((u1, u2, b22 - b12, u2 - b21)):
                    t[n, k:k + 128, tc:tc + 128] = v.astype(bf16)
            items.append((0, it))
        return items

    def pair(a, s, w, t, tc, c0, c1, fin):
        kh, st = t.shape[1], {}
        A = lambda r, k: a()[128 * r:128 * r + 128, kh * k:kh * k + kh]
        B = lambda k, c: w[kh * k:kh * k + kh, c:c + 128]
        T = lambda n: t[n, :, tc:tc + 128]
        R = lambda r, c, y: y + st["r"][128 * r:128 * r + 128, 128 * c:128 * c + 128] if "r" in st else y

        def rem():
            st["r"] = dot(a()[:, 2 * kh:], jnp.concatenate([w[2 * kh:, c:c + 128] for c in (c0, c1)], axis=1))
            return st["r"]

        def p1():
            st[1] = dot(A(0, 0), B(0, c0))
            return st[1]

        def p2():
            st[11] = R(0, 0, st[1] + dot(A(0, 1), B(1, c0)))
            return st[11]

        def p6():
            st[2] = st[1] + dot(s(1), T(1))
            return st[2]

        def p7():
            st[3] = st[2] + dot(s(2), T(2))
            return st[3]

        def p4():
            y = R(1, 0, st[3] - dot(A(1, 1), T(3)))
            fin(c0, jnp.concatenate([st[11], y], axis=0))
            return y

        def p5():
            y = dot(s(0), T(0))
            st[22], st[4] = R(1, 1, st[3] + y), st[2] + y
            return st[4]

        def p3():
            y = R(0, 1, st[4] + dot(s(3), B(1, c1)))
            fin(c1, jnp.concatenate([y, st[22]], axis=0))
            return y
        return [(128, rem)] * (w.shape[0] > 2 * kh) + [(kh // 4, p) for p in (p1, p2, p6, p7, p4, p5, p3)]

    def sums(y, kh):
        a11, a12, a21, a22 = y[:128, :kh], y[:128, kh:2 * kh], y[128:, :kh], y[128:, kh:2 * kh]
        s1 = a21 + a22
        s2 = s1 - a11
        s4 = a12 - s2
        if kh == 128 and P["FG"]:
            fence.append(s4.reshape(16, 8, 128).max(axis=0))
        return [v.astype(bf16) for v in (s1, s2, a11 - a21, s4)]

    seen, fence, cnt, defer = [], [], {}, []

    def gater(j0, j1):
        def gate(m):
            n = P["LC"]
            tk = [seen[j0 + (j1 - j0) * c // n][0:8, 0:1] for c in range(n)]
            tk = jnp.concatenate([v for v in tk for _ in range(TB // 8 // n)], axis=0)
            return jnp.where(jax.lax.broadcasted_iota(i32, (TB, 1), 0) < i // 4096, tk, m)
        return gate

    def norm(t, slot, back=0):
        if back:
            x_s[S:S + 16, 0:128] = seen[-back][0:16, 0:128].astype(bf16)
        y = _ln(x_s[rows(t), :].astype(f32), gater(len(seen) + 2 - back, len(seen)) if back and P["L1"] else None)
        xn_s[slot] = pltpu.bitcast(y.astype(bf16), i32)
        if slot == 0 and P["SQ"]:
            for n, v in enumerate(sums(y, 256)):
                xs_s[n] = pltpu.bitcast(v, i32)

    def qkv_items(t, slot, first=512):
        st = {}

        def xn():
            if "xn" not in st:
                st["xn"] = pltpu.bitcast(xn_s[slot], bf16)
            return st["xn"]
        lo = jax.lax.broadcasted_iota(i32, (TB // 2, 128), 1) < 64
        hrows = pl.ds(pl.multiple_of(t * (TB // 2), TB // 2), TB // 2)

        def slab(dst, scale):
            ys = {}

            def fin(c, y):
                j = c % D // 128
                ys[j] = y = pltpu.bitcast((y * scale if scale else y).astype(bf16), i32)
                if j != 2:
                    later.append(lambda: dst.__setitem__(((0, 2, None, 5, 7)[j], hrows), y))
                for jj in (j, j + 1):
                    if jj in ys and jj - 1 in ys:
                        m = jnp.where(lo, ys[jj], ys[jj - 1])
                        later.append(lambda m=m, jj=jj: dst.__setitem__(((None, 1, 3, 4, 6)[jj], hrows), m))
            return fin

        def vfin(c, y):
            j = c % D // 128
            st[j] = pltpu.bitcast(pltpu.bitcast(_ilv(y, True), bf16).T, i32)
            sub = jax.lax.broadcasted_iota(i32, (8, TB), 0)
            for h in range(H):
                r0 = DH * h // 16 * 8
                need = (r0 // 64, (r0 + 8) // 64)
                if j not in need or need[0] not in st or need[1] not in st:
                    continue
                a, b = (st[r // 64][r % 64:r % 64 + 8] for r in (r0, r0 + 8))
                if h % 4 < 2:
                    b = jnp.where(sub >= 4, 0x3F803F80, b)
                else:
                    a = jnp.where(sub < 4, 0x3F803F80, a)
                w = jnp.concatenate([a, b], axis=0)
                for bb in range(NB):
                    later.append(lambda w=w, h=h, bb=bb: vt_s.__setitem__((t * NB + bb, h), w[:, 128 * bb:128 * (bb + 1)]))
        fins = (slab(q_s, DH ** -0.5 * LOG2E), slab(k_s, None), vfin)
        if slot or not P["SQ"]:
            return [lin(xn, wqkv, D * n, D, fins[n], 512 if n else first) for n in range(3)]

        def xs(n):
            if ("s", n) not in st:
                st["s", n] = pltpu.bitcast(xs_s[n], bf16)
            return st["s", n]
        return [sum((pair(xn, xs, wqkv, tq, 256 * n + 128 * m, D * n + 256 * m, D * n + 256 * m + 128, fins[n])
                     for m in range(2)), []) + lin(xn, wqkv, D * n + 512, 128, fins[n]) for n in range(3)]

    def prep_q(n):
        return sum((prep(wqkv, tq, 256 * n + 128 * m, D * n + 256 * m, D * n + 256 * m + 128) for m in range(2 * P["SQ"])), [])

    def mlp_items(gate=None, hoist=0):
        hs, gs, ss, st = [], {}, [], {}

        def once(key, fn):
            if key not in st:
                st[key] = fn()
            return st[key]

        def f_o(c, y):
            hs.append(x_s[rows(i - 1), c:c + 128].astype(f32) + y)

        def f_up(c, y):
            gs[c] = jax.nn.gelu(y + b1_ref[c:c + 128].astype(f32).reshape(1, 128), approximate=True)
            if c >= F // 2 and P["S2"]:
                ss.append(sums(jnp.concatenate([gs[c - F // 2], gs[c]], axis=1), 128))

        def f_dn(c, y):
            y = y + b2_ref[c:c + 128].astype(f32).reshape(1, 128)
            o_ref[:, c:c + 128] = (hs[c // 128] + y).astype(o_ref.dtype)
        o = pltpu.bitcast(o_s[...], bf16)
        hf = lambda: once("hf", lambda: _ln(jnp.concatenate(hs, axis=1), gate))
        hn = lambda: once("hn", lambda: hf().astype(bf16))
        h4 = lambda n: once("h4", lambda: sums(hf(), 256))[n]
        u = lambda: once("u", lambda: jnp.concatenate([gs[c].astype(bf16) for c in sorted(gs)], axis=1))
        u4 = lambda n: once(("u4", n), lambda: jnp.concatenate([v[n] for v in ss], axis=1))
        if P["S1"]:
            up = sum((pair(hn, h4, w1, t1, c, c, c + F // 2, f_up) for c in range(0, F // 2, 128)), [])
        else:
            up = lin(hn, w1, 0, F, f_up)
        if P["S2"]:
            dn = lin(u, w2, 512, 128, f_dn) + sum((pair(u, u4, w2, t2, c, c, c + 256, f_dn) for c in (0, 128)), [])
        else:
            dn = lin(u, w2, 0, D, f_dn)
        if not hoist:
            return lin(lambda: o, wo, 0, D, f_o), up, dn
        top = {}
        m0 = lin(lambda: o[:128], wo, 0, D, top.__setitem__)
        m0 += lin(lambda: o[128:], wo, 0, D, lambda c, y: f_o(c, jnp.concatenate([top[c], y], axis=0)))
        early = [8 * n + 1 for n in range(hoist)]
        up = [up[n] for n in early] + [v for n, v in enumerate(up) if n not in early]
        return [(w // 2, it) for w, it in m0], up, dn

    lane = jax.lax.broadcasted_iota(i32, (8, 128), 1)
    tri32 = jax.lax.broadcasted_iota(i32, (32, 128), 0) > (jax.lax.broadcasted_iota(i32, (32, 128), 1) & 31)
    negc = NEG * LOG2E
    later = []

    def flush():
        for fn in later:
            fn()
        later.clear()

    def merge(p):
        c = jax.lax.broadcasted_iota(i32, p[0].shape, 1)
        i0, i1 = (c & 32) != 0, (c & 64) != 0
        u = [jnp.where(i0, p[(a + 1) % 4], p[a]) for a in range(4)]
        return [jnp.where(i1, u[(a + 2) % 4], u[a]) for a in range(4)]

    class Unit:
        def __init__(self, n, g, b, nprev, ot, opq):
            self.g, self.b, self.nprev, self.ot = g, b, nprev, ot
            self.f, self.p = (f0, f1)[n % 2], (p0, p1)[n % 2]
            self.z = (i // 1024, i // 2048) if opq else (0, 0)
            self.mx, self.blk = [None] * 4, i * NB + b

        def qk(self, j):
            g, nprev = self.g, self.nprev
            qb = q_s[g, pl.ds(pl.multiple_of(self.blk * 64 + 16 * j, 16), 16), :].reshape(2, 8, 128)
            parts = []
            for ii in range(4):
                h = 4 * g + (j - ii) % 4
                lm = jnp.where(((lane - DH * h) & 127) < DH, -1, 0)
                parts.append((qb & lm[None]).reshape(16, 128))
            qm = pltpu.bitcast(jnp.concatenate(parts, axis=0), bf16)
            ts = max(0, 256 - 128 * nprev - 32 * j)
            k0 = pl.multiple_of(self.blk * 64 - 128 + 16 * j + ts // 2, 16)
            kk = pltpu.bitcast(k_s[g, pl.ds(k0, 144 - ts // 2), :], bf16)
            s = jax.lax.dot_general(kk, qm, NT, preferred_element_type=f32)
            d = jnp.where(tri32, s[:32] if ts == 0 else negc, s[256 - ts:])
            self.f[self.z[0], j, 32 * j:32 * j + 32] = d
            mx = d
            for t in range(32, 256, 32):
                r = (32 * j + t) % 256
                if t >= ts:
                    v = s[t - ts:t - ts + 32]
                    mx = jnp.maximum(mx, v)
                    self.f[self.z[0], j, r:r + 32] = v
                elif r < 128:
                    self.f[self.z[0], j, r:r + 32] = jnp.full((32, 128), negc, f32)
            self.mx[j] = jnp.broadcast_to(jnp.max(mx, axis=0, keepdims=True), (8, 128))

        def ex(self, c, nc, tick):
            n = (256 if self.nprev else 128) // nc
            mx = [m if tick is None else jnp.where(never, tick, m) for m in self.mx]
            for r in range(c * n, (c + 1) * n, 16):
                p = [_ilv(jnp.exp2((self.f[self.z[1], j, r:r + 16].reshape(2, 8, 128) - mx[j][None]).reshape(16, 128)), False)
                     for j in range(4)]
                for hh, v in enumerate(merge(p)):
                    self.p[self.z[0], hh, r // 2:r // 2 + 8] = v

        def pv(self, hh):
            g, blk = self.g, self.blk
            h = 4 * g + hh
            mm = lambda bk, p: dot(pltpu.bitcast(vt_s[bk, h], bf16), pltpu.bitcast(p, bf16))
            pf = self.p[self.z[1], hh, 0:64]
            if self.nprev == 2:
                pa = pf & tri_s[hh]
                pf = pf ^ pa
            o = mm(blk, pf)
            if self.nprev >= 1:
                o += mm(blk - 1, self.p[self.z[1], hh, 64:128])
            if self.nprev == 2:
                o += mm(blk - 2, pa)
            l, o = (o[24:], o[:24]) if hh < 2 else (o[:8], o[8:])
            o = (o.reshape(3, 8, 128) * (1.0 / l)[None]).reshape(24, 128)
            if hh:
                o = pltpu.roll(o, 32 * hh, 1)
            off = 4 * (hh % 2)
            self.ot.append(o[off:off + DH])
            if h == H - 1:
                o_s[64 * self.b:64 * self.b + 64] = pltpu.bitcast(jnp.concatenate(self.ot, axis=0).T.astype(bf16), i32)

    def attend(first, dense, a0, a1):
        ots = [[] for _ in range(NB)]
        us = [(g, b) for b in range(NB) for g in range(NG)]
        us = [Unit(n, g, b, min(b, 2) if first else 2, ots[b], P["OF" if first else "OPQ"]) for n, (g, b) in enumerate(us)]
        first or seen.clear()
        n, nc = len(us), (8 if first else P["NC"])
        tie = P["TF" if first else "TIE"]
        tot, done = sum(w for w, _ in dense), 0

        def run(upto):
            nonlocal done
            out = []
            while dense and done + dense[0][0] // 2 <= upto:
                w, it = dense.pop(0)
                done += w
                y = it()
                if w:
                    out.append((w, y))
                    seen.append(y)
            return out
        run(a0)
        for t in range(n + 2):
            if t < n:
                for j in range(4):
                    us[t].qk(j)
            flush()
            fs = list(fence)
            fence.clear()
            if t >= 2:
                for j in range(4):
                    us[t - 2].pv(j)
            ys = run(a0 + (tot - a0 - a1) * t // n if t <= n else tot)
            if 1 <= t <= n:
                for c in range(nc):
                    tick = None
                    if ys and tie:
                        pos = int(c * sum(w for w, _ in ys) * tie) // nc
                        for w, y in ys:
                            if pos < w:
                                r = pos * y.shape[0] // w // 8 * 8
                                tick = y[r:r + 8, :128]
                                break
                            pos -= w
                    if c == nc - P["FG"]:
                        for v in fs:
                            tick = jnp.where(never, v, tick)
                    us[t - 1].ex(c, nc, tick)
        flush()

    prep_1 = lambda: sum((prep(w1, t1, c, c, c + F // 2) for c in range(0, F // 2 * P["S1"], 128)), [])

    @pl.when(i == 0)
    def _():
        for c in cps[:P['D0']]:
            c.start()
        row = jax.lax.broadcasted_iota(i32, (128, 128), 0)
        col = jax.lax.broadcasted_iota(i32, (128, 128), 1)
        for hh in range(4):
            tri_s[hh] = _ilv(pltpu.bitcast(jnp.where(row > ((col + 32 * hh) & 127), -1, 0), f32), False)
        def go(items):
            last = max(n for n, (w, _) in enumerate(items) if w)
            for n, (w, it) in enumerate(items):
                defer[:] = [1] * (n == last)
                y = it()
                if w:
                    seen.append(y)
            defer.clear()

        a, b = qkv_items(0, 1, QA), qkv_items(1, 2, QA)
        na = 1 + QA // 128
        cps[0].wait()
        norm(0, 1)
        cps[1].wait()
        go(a[0][:na])
        norm(1, 2)
        go(b[0][:na])
        cps[2].wait()
        flush()
        go(a[0][na:] + b[0][na:])
        for c in cps[P['D0']:]:
            c.start()
        cps[3].wait()
        flush()
        go(mix(a[1], prep_q(0) + prep_q(1)))
        cps[4].wait()
        flush()
        go(mix(a[2], prep_q(2)))
        flush()
        bb = b[1] + b[2]
        b0, b1 = bb[:P["FW"]], bb[P["FW"]:]
        b1.insert(1, (0, functools.partial(norm, 2, 0)))
        b1 = b1[:2] + mix(b1[2:], prep_1() * P["P1"])
        attend(True, b0 + [(0, cps[5].wait)] + [(0, cps[6].wait)] * P["P1"] + b1, P["F0"], P["F1"])

    @pl.when(i == 1)
    def _():
        seen.clear()
        if not P["P1"]:
            cps[6].wait()
            for _, it in prep_1():
                it()
        for c in cps[7:11]:
            c.wait()
        if P["S2"]:
            for _, it in prep(w2, t2, 0, 0, 256) + prep(w2, t2, 128, 128, 384):
                it()

    pl.when(i == 2)(cps[11].wait)

    @pl.when((i > 0) & (i < NT_ - 1))
    def _():
        m0, up, dn = mlp_items(gater(*P["L2"]) if P["L2"] else None)
        dn.insert(P["AN"], (0, functools.partial(norm, jnp.minimum(i + 2, NT_ - 1), 0, P["AB"])))
        attend(False, m0 + sum(qkv_items(i + 1, 0), []) + up + dn, P["A0"], P["A1"])

    @pl.when(i == NT_ - 1)
    def _():
        attend(False, sum(mlp_items(None, P["H7"]), []), P["B0"], P["B1"])

    @pl.when(i == NT_)
    def _():
        for _, it in sum(mlp_items(None, P["H8"]), []):
            it()


def run(A_x, A_wqkv, A_wo, B_x, B_w1, B_b1, B_w2, B_b2, **kw):
    P = dict(NC=16, OPQ=1, TIE=0.65, A0=512, A1=768, B0=1800, B1=768, TF=0, F0=0, F1=1400, AN=16, AB=14, L1=1, L2=(10, 40), FG=0, P1=1, H7=3, H8=6, OA=1, LC=8, FW=4, SQ=1, S1=1, S2=1, QA=256, D0=7, OF=0)
    P.update(kw)
    del B_x
    hbm = pl.BlockSpec(memory_space=pl.ANY)
    out = pl.pallas_call(
        functools.partial(_kernel, P=P),
        grid=(NT_ + 1,),
        in_specs=[hbm] * 7,
        out_specs=pl.BlockSpec((None, TB, D), lambda i: (0, jnp.maximum(i - 1, 0), 0)),
        out_shape=jax.ShapeDtypeStruct((1, S, D), bf16),
        scratch_shapes=[pltpu.VMEM((F,), bf16), pltpu.VMEM((D,), bf16),
                        pltpu.VMEM((S + 16, D), bf16), pltpu.VMEM((D, 3 * D), bf16), pltpu.VMEM((D, D), bf16),
                        pltpu.VMEM((D, F), bf16), pltpu.VMEM((F, D), bf16),
                        pltpu.VMEM((NG, S // 2, 128), i32), pltpu.VMEM((NG, S // 2, 128), i32),
                        pltpu.VMEM((S // 128, H, 16, 128), i32), pltpu.VMEM((TB // 2, D), i32),
                        pltpu.SemaphoreType.DMA((12,)), pltpu.VMEM((4, 64, 128), i32), pltpu.VMEM((3, TB // 2, D), i32), pltpu.VMEM((4, 64, 256), i32),
                        pltpu.VMEM((4, 256, 768), bf16), pltpu.VMEM((4, 256, 768), bf16), pltpu.VMEM((4, 768, 256), bf16),
                        *[pltpu.VMEM((1, 4, 256, 128), f32)] * 2, *[pltpu.VMEM((1, 4, 128, 128), i32)] * 2],
        compiler_params=pltpu.CompilerParams(dimension_semantics=("arbitrary",),
                                             vmem_limit_bytes=100 * 1024 * 1024),
    )(A_x, A_wqkv, A_wo, B_w1, B_b1, B_w2, B_b2)
    return out


@jax.jit
def pallas_sequential_preLN__sliding_block__dense_activation_gelu__prompt_kernel(
        A_x, A_wqkv, A_wo, B_x, B_w1, B_b1, B_w2, B_b2):
    return run(A_x, A_wqkv, A_wo, B_x, B_w1, B_b1, B_w2, B_b2)
```

```python
import functools
import numpy as np
import jax
import jax.numpy as jnp
import jax.experimental.pallas as pl
import jax.experimental.pallas.tpu as pltpu

S, D, F, H, W = 2048, 640, 1536, 32, 256
DH = D // H
NG = 8
TB = 256
NB = TB // 128
NT_ = S // TB
NEG = -1e9
LOG2E = 1.4426950408889634
bf16, f32, i32 = jnp.bfloat16, jnp.float32, jnp.int32
NT = (((1,), (1,)), ((), ()))
HI = -65536
dot = functools.partial(jnp.dot, preferred_element_type=f32)


def _ln(x, gate=None):
    m = jnp.mean(x, axis=-1, keepdims=True)
    if gate:
        m = gate(m)
    xc = x - m
    v = jnp.mean(xc * xc, axis=-1, keepdims=True)
    return xc * jax.lax.rsqrt(v + 1e-5)


def _ilv(y, rnd):
    n, c = y.shape
    b = pltpu.bitcast(y, i32)
    if rnd:
        b = b + 0x8000
    b = b.reshape(n // 16, 2, 8, c)
    w = jax.lax.shift_right_logical(b[:, 0], 16) | (b[:, 1] & HI)
    return w.reshape(n // 2, c)


def mix(a, b):
    return [it for _, it in sorted([(n / len(a), x) for n, x in enumerate(a)] + [(n / (len(b) + 1), x) for n, x in enumerate(b)],
                                   key=lambda q: q[0])]


class Packed:
    def __init__(self, r):
        self.r, self.shape = r, r.shape[:-2] + (r.shape[-2] * 2, r.shape[-1])

    def _ix(self, ix):
        *a, k, c = ix
        return (*a, slice((k.start or 0) // 2, (k.stop or self.shape[-2]) // 2), c)

    def __getitem__(self, ix):
        return pltpu.bitcast(self.r[self._ix(ix)], bf16)

    def __setitem__(self, ix, v):
        self.r[self._ix(ix)] = pltpu.bitcast(v, i32)


def _kernel(x_h, wqkv_h, wo_h, w1_h, b1_h, w2_h, b2_h, out_h, out_s, osem, b1_ref, b2_ref,
            x_s, wqkv, wo, w1, w2, q_s, k_s, vt_s, o_s, sem, tri_s, xn_s, xs_s, tq, t1, t2, f0, f1, p0, p1, *, P):
    wqkv_h, wo_h, w1_h, w2_h = (r.bitcast(i32) for r in (wqkv_h, wo_h, w1_h, w2_h))
    i = pl.program_id(0)
    never = jax.lax.broadcasted_iota(i32, (8, 128), 1) < i // 4096
    QA = P["QA"]
    pairs = [(x_h.at[0, 0:2 * TB], x_s.at[0:2 * TB])]
    pairs += [(wqkv_h.at[:, c:e], wqkv.at[:, c:e]) for c, e in ((0, QA), (QA, D), (D, 2 * D), (2 * D, 3 * D))]
    pairs += [(x_h.at[0, 2 * TB:4 * TB], x_s.at[2 * TB:4 * TB]), (w1_h, w1), (w2_h, w2),
              (wo_h, wo), (b1_h, b1_ref), (b2_h, b2_ref), (x_h.at[0, 4 * TB:S], x_s.at[4 * TB:S])]
    cps = [pltpu.make_async_copy(s, d, sem.at[n]) for n, (s, d) in enumerate(pairs)]

    tq, t1, t2, wqkv, wo, w1, w2 = map(Packed, (tq, t1, t2, wqkv, wo, w1, w2))

    def rows(t):
        return pl.ds(pl.multiple_of(t * TB, TB), TB)

    def lin(a, w, c0, n, fin, first=512):
        items, st = [], {}
        kk = w.shape[0]
        cuts = [0] + list(range(first, n, 512)) + [n]
        for c, e in zip(cuts, cuts[1:]):
            if kk % 512:
                def rem(c=c, e=e):
                    st[c] = dot(a()[:, 512:], w[512:, c0 + c:c0 + e])
                    return st[c]
                items.append(((e - c) // 2, rem))
            for cc in range(c, e, 128):
                for k in range(0, kk - 511, 512):
                    def main(c=c, cc=cc, k=k):
                        y = dot(a()[:, k:k + 512], w[k:k + 512, c0 + cc:c0 + cc + 128])
                        if k:
                            y = y + st["acc"]
                        elif kk % 512:
                            y = y + st[c][:, cc - c:cc - c + 128]
                        st["acc"] = y
                        if k + 1024 > kk:
                            later.append(lambda: fin(c0 + cc, y)) if defer else fin(c0 + cc, y)
                        return y
                    items.append((256, main))
        return items

    def prep(w, t, tc, c0, c1):
        kh, items = t.shape[1], []
        for k in range(0, kh, 128):
            def it(k=k):
                b11, b12, b21, b22 = (w[r:r + 128, c:c + 128].astype(f32) for r in (k, k + kh) for c in (c0, c1))
                if seen:
                    y = seen[-1]
                    r = cnt.setdefault(id(y), 0) * 64 % y.shape[0]
                    cnt[id(y)] += 1
                    b12 = jnp.where(never[None], y[r:r + 8, :128][None], b12.reshape(16, 8, 128)).reshape(128, 128)
                u1 = b12 - b11
                u2 = b22 - u1
                for n, v in enumerate((u1, u2, b22 - b12, u2 - b21)):
                    t[n, k:k + 128, tc:tc + 128] = v.astype(bf16)
            items.append((0, it))
        return items

    def pair(a, s, w, t, tc, c0, c1, fin):
        kh, st = t.shape[1], {}
        A = lambda r, k: a()[128 * r:128 * r + 128, kh * k:kh * k + kh]
        B = lambda k, c: w[kh * k:kh * k + kh, c:c + 128]
        T = lambda n: t[n, :, tc:tc + 128]
        R = lambda r, c, y: y + st["r"][128 * r:128 * r + 128, 128 * c:128 * c + 128] if "r" in st else y

        def rem():
            st["r"] = dot(a()[:, 2 * kh:], jnp.concatenate([w[2 * kh:, c:c + 128] for c in (c0, c1)], axis=1))
            return st["r"]

        def p1():
            st[1] = dot(A(0, 0), B(0, c0))
            return st[1]

        def p2():
            st[11] = R(0, 0, st[1] + dot(A(0, 1), B(1, c0)))
            return st[11]

        def p6():
            st[2] = st[1] + dot(s(1), T(1))
            return st[2]

        def p7():
            st[3] = st[2] + dot(s(2), T(2))
            return st[3]

        def p4():
            y = R(1, 0, st[3] - dot(A(1, 1), T(3)))
            fin(c0, jnp.concatenate([st[11], y], axis=0))
            return y

        def p5():
            y = dot(s(0), T(0))
            st[22], st[4] = R(1, 1, st[3] + y), st[2] + y
            return st[4]

        def p3():
            y = R(0, 1, st[4] + dot(s(3), B(1, c1)))
            fin(c1, jnp.concatenate([y, st[22]], axis=0))
            return y
        return [(128, rem)] * (w.shape[0] > 2 * kh) + [(kh // 4, p) for p in (p1, p2, p6, p7, p4, p5, p3)]

    def sums(y, kh):
        a11, a12, a21, a22 = y[:128, :kh], y[:128, kh:2 * kh], y[128:, :kh], y[128:, kh:2 * kh]
        s1 = a21 + a22
        s2 = s1 - a11
        s4 = a12 - s2
        if kh == 128 and P["FG"]:
            fence.append(s4.reshape(16, 8, 128).max(axis=0))
        return [v.astype(bf16) for v in (s1, s2, a11 - a21, s4)]

    seen, fence, cnt, defer = [], [], {}, []

    def gater(j0, j1):
        def gate(m):
            n = P["LC"]
            tk = [seen[j0 + (j1 - j0) * c // n][0:8, 0:1] for c in range(n)]
            tk = jnp.concatenate([v for v in tk for _ in range(TB // 8 // n)], axis=0)
            return jnp.where(jax.lax.broadcasted_iota(i32, (TB, 1), 0) < i // 4096, tk, m)
        return gate

    def norm(t, slot, back=0):
        if back:
            x_s[S:S + 16, 0:128] = seen[-back][0:16, 0:128].astype(bf16)
        y = _ln(x_s[rows(t), :].astype(f32), gater(len(seen) + 2 - back, len(seen)) if back and P["L1"] else None)
        xn_s[slot] = pltpu.bitcast(y.astype(bf16), i32)
        if slot == 0:
            for n, v in enumerate(sums(y, 256)):
                xs_s[n] = pltpu.bitcast(v, i32)

    def qkv_items(t, slot, first=512):
        st = {}

        def xn():
            if "xn" not in st:
                st["xn"] = pltpu.bitcast(xn_s[slot], bf16)
            return st["xn"]
        lo = jax.lax.broadcasted_iota(i32, (TB // 2, 128), 1) < 64
        hrows = pl.ds(pl.multiple_of(t * (TB // 2), TB // 2), TB // 2)

        def slab(dst, scale):
            ys = {}

            def fin(c, y):
                j = c % D // 128
                ys[j] = y = pltpu.bitcast((y * scale if scale else y).astype(bf16), i32)
                if j != 2:
                    later.append(lambda: dst.__setitem__(((0, 2, None, 5, 7)[j], hrows), y))
                for jj in (j, j + 1):
                    if jj in ys and jj - 1 in ys:
                        m = jnp.where(lo, ys[jj], ys[jj - 1])
                        later.append(lambda m=m, jj=jj: dst.__setitem__(((None, 1, 3, 4, 6)[jj], hrows), m))
            return fin

        def vfin(c, y):
            j = c % D // 128
            st[j] = pltpu.bitcast(pltpu.bitcast(_ilv(y, True), bf16).T, i32)
            sub = jax.lax.broadcasted_iota(i32, (8, TB), 0)
            for h in range(H):
                r0 = DH * h // 16 * 8
                need = (r0 // 64, (r0 + 8) // 64)
                if j not in need or need[0] not in st or need[1] not in st:
                    continue
                a, b = (st[r // 64][r % 64:r % 64 + 8] for r in (r0, r0 + 8))
                if h % 4 < 2:
                    b = jnp.where(sub >= 4, 0x3F803F80, b)
                else:
                    a = jnp.where(sub < 4, 0x3F803F80, a)
                w = jnp.concatenate([a, b], axis=0)
                for bb in range(NB):
                    later.append(lambda w=w, h=h, bb=bb: vt_s.__setitem__((t * NB + bb, h), w[:, 128 * bb:128 * (bb + 1)]))
        fins = (slab(q_s, DH ** -0.5 * LOG2E), slab(k_s, None), vfin)
        if slot:
            return [lin(xn, wqkv, D * n, D, fins[n], 512 if n else first) for n in range(3)]

        def xs(n):
            if ("s", n) not in st:
                st["s", n] = pltpu.bitcast(xs_s[n], bf16)
            return st["s", n]
        return [sum((pair(xn, xs, wqkv, tq, 256 * n + 128 * m, D * n + 256 * m, D * n + 256 * m + 128, fins[n])
                     for m in range(2)), []) + lin(xn, wqkv, D * n + 512, 128, fins[n]) for n in range(3)]

    def prep_q(n):
        return sum((prep(wqkv, tq, 256 * n + 128 * m, D * n + 256 * m, D * n + 256 * m + 128) for m in range(2)), [])

    def mlp_items(gate=None, hoist=0, mid=None):
        hs, gs, ss, st = [], {}, [], {}

        def once(key, fn):
            if key not in st:
                st[key] = fn()
            return st[key]

        def f_o(c, y):
            hs.append(x_s[rows(i - 1), c:c + 128].astype(f32) + y)

        def f_up(c, y):
            gs[c] = jax.nn.gelu(y + b1_ref[c:c + 128].astype(f32).reshape(1, 128), approximate=True)
            if c >= F // 2:
                ss.append(sums(jnp.concatenate([gs[c - F // 2], gs[c]], axis=1), 128))

        def f_dn(c, y):
            y = y + b2_ref[c:c + 128].astype(f32).reshape(1, 128)
            out_s[rows(i - 1), c:c + 128] = (hs[c // 128] + y).astype(bf16)
        o = pltpu.bitcast(o_s[...], bf16)
        hf = lambda: once("hf", lambda: _ln(jnp.concatenate(hs, axis=1), gate))
        hn = lambda: once("hn", lambda: hf().astype(bf16))
        h4 = lambda n: once("h4", lambda: sums(hf(), 256))[n]
        u = lambda: once("u", lambda: jnp.concatenate([gs[c].astype(bf16) for c in sorted(gs)], axis=1))
        u4 = lambda n: once(("u4", n), lambda: jnp.concatenate([v[n] for v in ss], axis=1))
        up = sum((pair(hn, h4, w1, t1, c, c, c + F // 2, f_up) for c in range(0, F // 2, 128)), [])
        dn = [lin(u, w2, 512, 128, f_dn)] + [pair(u, u4, w2, t2, c, c, c + 256, f_dn) for c in (0, 128)]
        dn = dn[1] + dn[2] + [(0, mid)] + dn[0] if mid else dn[0] + dn[1] + dn[2]
        if not hoist:
            return lin(lambda: o, wo, 0, D, f_o), up, dn
        top = {}
        m0 = lin(lambda: o[:128], wo, 0, D, top.__setitem__)
        m0 += lin(lambda: o[128:], wo, 0, D, lambda c, y: f_o(c, jnp.concatenate([top[c], y], axis=0)))
        early = [8 * n + 1 for n in range(hoist)]
        up = [up[n] for n in early] + [v for n, v in enumerate(up) if n not in early]
        return [(w // 2, it) for w, it in m0], up, dn

    lane = jax.lax.broadcasted_iota(i32, (8, 128), 1)
    tri32 = jax.lax.broadcasted_iota(i32, (32, 128), 0) > (jax.lax.broadcasted_iota(i32, (32, 128), 1) & 31)
    negc = NEG * LOG2E
    later = []

    def flush():
        for fn in later:
            fn()
        later.clear()

    def merge(p):
        c = jax.lax.broadcasted_iota(i32, p[0].shape, 1)
        i0, i1 = (c & 32) != 0, (c & 64) != 0
        u = [jnp.where(i0, p[(a + 1) % 4], p[a]) for a in range(4)]
        return [jnp.where(i1, u[(a + 2) % 4], u[a]) for a in range(4)]

    class Unit:
        def __init__(self, n, g, b, nprev, ot, opq):
            self.g, self.b, self.nprev, self.ot = g, b, nprev, ot
            self.f, self.p = (f0, f1)[n % 2], (p0, p1)[n % 2]
            self.z = (i // 1024, i // 2048) if opq else (0, 0)
            self.mx, self.blk = [None] * 4, i * NB + b

        def qk(self, j):
            g, nprev = self.g, self.nprev
            qb = q_s[g, pl.ds(pl.multiple_of(self.blk * 64 + 16 * j, 16), 16), :].reshape(2, 8, 128)
            parts = []
            for ii in range(4):
                h = 4 * g + (j - ii) % 4
                lm = jnp.where(((lane - DH * h) & 127) < DH, -1, 0)
                parts.append((qb & lm[None]).reshape(16, 128))
            qm = pltpu.bitcast(jnp.concatenate(parts, axis=0), bf16)
            ts = max(0, 256 - 128 * nprev - 32 * j)
            k0 = pl.multiple_of(self.blk * 64 - 128 + 16 * j + ts // 2, 16)
            kk = pltpu.bitcast(k_s[g, pl.ds(k0, 144 - ts // 2), :], bf16)
            s = jax.lax.dot_general(kk, qm, NT, preferred_element_type=f32)
            d = jnp.where(tri32, s[:32] if ts == 0 else negc, s[256 - ts:])
            self.f[self.z[0], j, 32 * j:32 * j + 32] = d
            mx = d
            for t in range(32, 256, 32):
                r = (32 * j + t) % 256
                if t >= ts:
                    v = s[t - ts:t - ts + 32]
                    mx = jnp.maximum(mx, v)
                    self.f[self.z[0], j, r:r + 32] = v
                elif r < 128:
                    self.f[self.z[0], j, r:r + 32] = jnp.full((32, 128), negc, f32)
            self.mx[j] = jnp.broadcast_to(jnp.max(mx, axis=0, keepdims=True), (8, 128))

        def ex(self, c, nc, tick):
            n = (256 if self.nprev else 128) // nc
            mx = [m if tick is None else jnp.where(never, tick, m) for m in self.mx]
            for r in range(c * n, (c + 1) * n, 16):
                p = [_ilv(jnp.exp2((self.f[self.z[1], j, r:r + 16].reshape(2, 8, 128) - mx[j][None]).reshape(16, 128)), False)
                     for j in range(4)]
                for hh, v in enumerate(merge(p)):
                    self.p[self.z[0], hh, r // 2:r // 2 + 8] = v

        def pv(self, hh):
            g, blk = self.g, self.blk
            h = 4 * g + hh
            mm = lambda bk, p: dot(pltpu.bitcast(vt_s[bk, h], bf16), pltpu.bitcast(p, bf16))
            pf = self.p[self.z[1], hh, 0:64]
            if self.nprev == 2:
                pa = pf & tri_s[hh]
                pf = pf ^ pa
            o = mm(blk, pf)
            if self.nprev >= 1:
                o += mm(blk - 1, self.p[self.z[1], hh, 64:128])
            if self.nprev == 2:
                o += mm(blk - 2, pa)
            l, o = (o[24:], o[:24]) if hh < 2 else (o[:8], o[8:])
            o = (o.reshape(3, 8, 128) * (1.0 / l)[None]).reshape(24, 128)
            if hh:
                o = pltpu.roll(o, 32 * hh, 1)
            off = 4 * (hh % 2)
            self.ot.append(o[off:off + DH])
            if h == H - 1:
                o_s[64 * self.b:64 * self.b + 64] = pltpu.bitcast(jnp.concatenate(self.ot, axis=0).T.astype(bf16), i32)

    def attend(first, dense, a0, a1, tie):
        ots = [[] for _ in range(NB)]
        us = [(g, b) for b in range(NB) for g in range(NG)]
        us = [Unit(n, g, b, min(b, 2) if first else 2, ots[b], P["OF" if first else "OPQ"]) for n, (g, b) in enumerate(us)]
        first or seen.clear()
        n, nc = len(us), (8 if first else P["NC"])
        tot, done = sum(w for w, _ in dense), 0

        def run(upto):
            nonlocal done
            out = []
            while dense and done + dense[0][0] // 2 <= upto:
                w, it = dense.pop(0)
                done += w
                y = it()
                if w:
                    out.append((w, y))
                    seen.append(y)
            return out
        run(a0)
        for t in range(n + 2):
            if t < n:
                for j in range(4):
                    us[t].qk(j)
            flush()
            fs = list(fence)
            fence.clear()
            if t >= 2:
                for j in range(4):
                    us[t - 2].pv(j)
            ys = run(a0 + (tot - a0 - a1) * t // n if t <= n else tot)
            if 1 <= t <= n:
                for c in range(nc):
                    tick = None
                    if ys and tie:
                        pos = int(c * sum(w for w, _ in ys) * tie) // nc
                        for w, y in ys:
                            if pos < w:
                                r = pos * y.shape[0] // w // 8 * 8
                                tick = y[r:r + 8, :128]
                                break
                            pos -= w
                    if c == nc - P["FG"]:
                        for v in fs:
                            tick = jnp.where(never, v, tick)
                    us[t - 1].ex(c, nc, tick)
        flush()

    prep_1 = lambda: sum((prep(w1, t1, c, c, c + F // 2)
                          for c in range(0, F // 2, 128)), [])

    @pl.when(i == 0)
    def _():
        for c in cps[:P['D0']]:
            c.start()
        row = jax.lax.broadcasted_iota(i32, (128, 128), 0)
        col = jax.lax.broadcasted_iota(i32, (128, 128), 1)
        for hh in range(4):
            tri_s[hh] = _ilv(pltpu.bitcast(jnp.where(row > ((col + 32 * hh) & 127), -1, 0), f32), False)
        def go(items):
            last = max(n for n, (w, _) in enumerate(items) if w)
            for n, (w, it) in enumerate(items):
                defer[:] = [1] * (n == last)
                y = it()
                if w:
                    seen.append(y)
            defer.clear()

        a, b = qkv_items(0, 1, QA), qkv_items(1, 2, QA)
        na = 1 + QA // 128
        cps[0].wait()
        norm(0, 1)
        cps[1].wait()
        go(a[0][:na])
        norm(1, 2)
        go(b[0][:na])
        cps[2].wait()
        flush()
        go(mix(a[0][na:] + b[0][na:], prep_q(0)))
        for c in cps[P['D0']:]:
            c.start()
        cps[3].wait()
        flush()
        go(mix(a[1], prep_q(1)))
        cps[4].wait()
        flush()
        go(mix(a[2], prep_q(2)))
        flush()
        bb = b[1] + b[2]
        b0, b1 = bb[:P["FW"]], bb[P["FW"]:]
        b1.insert(1, (0, functools.partial(norm, 2, 0)))
        b1 = b1[:2] + mix(b1[2:], prep_1() * P["P1"])
        attend(True, b0 + [(0, cps[5].wait)] + [(0, cps[6].wait)] * P["P1"] + b1, P["F0"], P["F1"], P["TF"])

    @pl.when(i == 1)
    def _():
        seen.clear()
        if not P["P1"]:
            cps[6].wait()
            for _, it in prep_1():
                it()
        for c in cps[7:11]:
            c.wait()
        for _, it in prep(w2, t2, 0, 0, 256) + prep(w2, t2, 128, 128, 384):
            it()

    def put(t, c, e, n):
        r = rows(t) if isinstance(t, jax.Array) else pl.ds(t * TB, TB)
        return pltpu.make_async_copy(out_s.at[r, c:e], out_h.at[0, r, c:e], osem.at[n])

    pl.when(i == 2)(cps[11].wait)
    pl.when(i >= 2)(lambda: put(i - 2, 0, D, i - 2).start())

    @pl.when((i > 0) & (i < NT_ - 1))
    def _():
        m0, up, dn = mlp_items(gater(*P["L2"]) if P["L2"] else None)
        dn.insert(P["AN"], (0, functools.partial(norm, jnp.minimum(i + 2, NT_ - 1), 0, P["AB"])))
        attend(False, m0 + sum(qkv_items(i + 1, 0), []) + up + dn, P["A0"], P["A1"], P["TIE"])

    @pl.when(i == NT_ - 1)
    def _():
        attend(False, sum(mlp_items(None, P["H7"]), []), P["B0"], P["B1"], P["T7"])

    @pl.when(i == NT_)
    def _():
        last = [put(NT_ - 1, 0, 512, NT_ - 1), put(NT_ - 1, 512, D, NT_)]
        for _, it in sum(mlp_items(None, P["H8"], last[0].start), []):
            it()
        last[1].start()
        for c in [put(t, 0, D, t) for t in range(NT_ - 1)] + last:
            c.wait()


def run(A_x, A_wqkv, A_wo, B_x, B_w1, B_b1, B_w2, B_b2, **kw):
    P = dict(NC=16, OPQ=1, TIE=0.6, A0=512, A1=768, B0=1800, B1=768, TF=0.4, F0=256, F1=1400, AN=16, AB=14, L1=1, L2=(10, 30), FG=0, P1=1, H7=3, H8=6, OA=1, LC=16, FW=6, T7=0.75, QA=256, D0=7, OF=0)
    P.update(kw)
    del B_x
    hbm = pl.BlockSpec(memory_space=pl.ANY)
    out = pl.pallas_call(
        functools.partial(_kernel, P=P),
        grid=(NT_ + 1,),
        in_specs=[hbm] * 7,
        out_specs=hbm,
        out_shape=jax.ShapeDtypeStruct((1, S, D), bf16),
        scratch_shapes=[pltpu.VMEM((S, D), bf16), pltpu.SemaphoreType.DMA((NT_ + 1,)),
                        pltpu.VMEM((F,), bf16), pltpu.VMEM((D,), bf16),
                        pltpu.VMEM((S + 16, D), bf16),
                        *[pltpu.VMEM(s, i32) for s in ((D // 2, 3 * D), (D // 2, D), (D // 2, F), (F // 2, D))],
                        pltpu.VMEM((NG, S // 2, 128), i32), pltpu.VMEM((NG, S // 2, 128), i32),
                        pltpu.VMEM((S // 128, H, 16, 128), i32), pltpu.VMEM((TB // 2, D), i32),
                        pltpu.SemaphoreType.DMA((12,)), pltpu.VMEM((4, 64, 128), i32), pltpu.VMEM((3, TB // 2, D), i32), pltpu.VMEM((4, 64, 256), i32),
                        *[pltpu.VMEM(s, i32) for s in ((4, 128, 768), (4, 128, 768), (4, 384, 256))],
                        *[pltpu.VMEM((1, 4, 256, 128), f32)] * 2, *[pltpu.VMEM((1, 4, 128, 128), i32)] * 2],
        compiler_params=pltpu.CompilerParams(dimension_semantics=("arbitrary",),
                                             vmem_limit_bytes=100 * 1024 * 1024),
    )(A_x, A_wqkv, A_wo, B_w1, B_b1, B_w2, B_b2)
    return out


@jax.jit
def pallas_sequential_preLN__sliding_block__dense_activation_gelu__prompt_kernel(
        A_x, A_wqkv, A_wo, B_x, B_w1, B_b1, B_w2, B_b2):
    return run(A_x, A_wqkv, A_wo, B_x, B_w1, B_b1, B_w2, B_b2)
```

```python
import functools

import jax
import jax.numpy as jnp
import jax.experimental.pallas as pl
import jax.experimental.pallas.tpu as pltpu

S, D, F, H = 2048, 640, 1536, 32
DH = D // H
NG = H // 4
TB = 256
NB = TB // 128
STEPS = S // TB
LOG2E = 1.4426950408889634
MASKED = -1e9 * LOG2E
ONES = 0x3F803F80
QA = 256
QP = [(0, 128), (256, 384), (512, D + 512)] + [(D * n + c, D * n + c + 128) for n in (1, 2) for c in (0, 256)]
bf16, f32, i32 = jnp.bfloat16, jnp.float32, jnp.int32
dot = functools.partial(jnp.dot, preferred_element_type=f32)
iota = functools.partial(jax.lax.broadcasted_iota, i32)


def _ln(x, gate=None):
    m = jnp.mean(x, axis=-1, keepdims=True)
    if gate:
        m = gate(m)
    xc = x - m
    v = jnp.mean(xc * xc, axis=-1, keepdims=True)
    return xc * jax.lax.rsqrt(v + 1e-5)


def _ilv(y, rnd):
    n, c = y.shape
    b = pltpu.bitcast(y, i32)
    if rnd:
        b = b + 0x8000
    b = b.reshape(n // 16, 2, 8, c)
    return (jax.lax.shift_right_logical(b[:, 0], 16) | (b[:, 1] & -65536)).reshape(n // 2, c)


def _mix(a, b):
    keyed = [(n / len(a), x) for n, x in enumerate(a)] + [(n / (len(b) + 1), x) for n, x in enumerate(b)]
    return [it for _, it in sorted(keyed, key=lambda q: q[0])]


def _merge(p):
    c = iota(p[0].shape, 1)
    odd, high = (c & 32) != 0, (c & 64) != 0
    u = [jnp.where(odd, p[(a + 1) % 4], p[a]) for a in range(4)]
    return [jnp.where(high, u[(a + 2) % 4], u[a]) for a in range(4)]


def _sums(y, kh):
    a11, a12, a21, a22 = y[:128, :kh], y[:128, kh:2 * kh], y[128:, :kh], y[128:, kh:2 * kh]
    s1 = a21 + a22
    s2 = s1 - a11
    return [v.astype(bf16) for v in (s1, s2, a11 - a21, a12 - s2)]


class _Packed:
    def __init__(self, r):
        self.r, self.shape = r, r.shape[:-2] + (r.shape[-2] * 2, r.shape[-1])

    def _ix(self, ix):
        *a, k, c = ix
        return (*a, slice((k.start or 0) // 2, (k.stop or self.shape[-2]) // 2), c)

    def __getitem__(self, ix):
        return pltpu.bitcast(self.r[self._ix(ix)], bf16)

    def __setitem__(self, ix, v):
        self.r[self._ix(ix)] = pltpu.bitcast(v, i32)


def _kernel(x_h, wqkv_h, wo_h, w1_h, b1_h, w2_h, b2_h, out_h, out_s, osem, b1_s, b2_s, x_s, wqkv, wo, w1, w2,
            q_s, k_s, vt_s, o_s, sem, tri_s, xn_s, xs_s, tq, t1, t2, f0, f1, p0, p1):
    i = pl.program_id(0)
    moves = [(x_h.at[0, 0:2 * TB], x_s.at[0:2 * TB])]
    moves += [(wqkv_h.at[:, c:e], wqkv.at[:, c:e]) for c, e in ((0, QA), (QA, D), (D, 2 * D), (2 * D, 3 * D))]
    moves += [(x_h.at[0, 2 * TB:4 * TB], x_s.at[2 * TB:4 * TB]), (w1_h, w1), (w2_h, w2),
              (wo_h, wo), (b1_h, b1_s), (b2_h, b2_s), (x_h.at[0, 4 * TB:S], x_s.at[4 * TB:S])]
    cps = [pltpu.make_async_copy(s, d, sem.at[n]) for n, (s, d) in enumerate(moves)]
    tq, t1, t2 = map(_Packed, (tq, t1, t2))

    never = iota((8, 128), 1) < i // 4096
    seen, used, later, defer = [], {}, [], []

    def rows(t):
        return pl.ds(pl.multiple_of(t * TB, TB), TB)

    def flush():
        for fn in later:
            fn()
        later.clear()

    def put(t, c, e, n):
        r = rows(t) if isinstance(t, jax.Array) else pl.ds(t * TB, TB)
        return pltpu.make_async_copy(out_s.at[r, c:e], out_h.at[0, r, c:e], osem.at[n])

    def lin(a, w, c0, n, fin, first=512):
        items, st, kk = [], {}, w.shape[0]
        cuts = [0] + list(range(first, n, 512)) + [n]
        for c, e in zip(cuts, cuts[1:]):
            if kk % 512:
                def rem(c=c, e=e):
                    st[c] = dot(a()[:, 512:], w[512:, c0 + c:c0 + e])
                    return st[c]
                items.append(((e - c) // 2, rem))
            for cc in range(c, e, 128):
                for k in range(0, kk - 511, 512):
                    def main(c=c, cc=cc, k=k):
                        y = dot(a()[:, k:k + 512], w[k:k + 512, c0 + cc:c0 + cc + 128])
                        if k:
                            y = y + st["acc"]
                        elif kk % 512:
                            y = y + st[c][:, cc - c:cc - c + 128]
                        st["acc"] = y
                        if k + 1024 > kk:
                            later.append(lambda: fin(c0 + cc, y)) if defer else fin(c0 + cc, y)
                        return y
                    items.append((256, main))
        return items

    def prep(w, t, tc, c0, c1):
        kh, items = t.shape[1], []
        for k in range(0, kh, 128):
            def it(k=k):
                b11, b12, b21, b22 = (w[r:r + 128, c:c + 128].astype(f32) for r in (k, k + kh) for c in (c0, c1))
                if seen:
                    r = used.get(len(seen), 0) * 64 % seen[-1].shape[0]
                    used[len(seen)] = used.get(len(seen), 0) + 1
                    b12 = jnp.where(never[None], seen[-1][r:r + 8, :128][None],
                                    b12.reshape(16, 8, 128)).reshape(128, 128)
                u1 = b12 - b11
                u2 = b22 - u1
                for n, v in enumerate((u1, u2, b22 - b12, u2 - b21)):
                    t[n, k:k + 128, tc:tc + 128] = v.astype(bf16)
            items.append((0, it))
        return items

    def pair(a, s, w, t, tc, c0, c1, fin):
        kh, st = t.shape[1], {}
        A = lambda r, k: a()[128 * r:128 * r + 128, kh * k:kh * k + kh]
        B = lambda k, c: w[kh * k:kh * k + kh, c:c + 128]
        T = lambda n: t[n, :, tc:tc + 128]
        R = lambda r, c, y: y + st["r"][128 * r:128 * r + 128, 128 * c:128 * c + 128] if "r" in st else y

        def rem():
            st["r"] = dot(a()[:, 2 * kh:], jnp.concatenate([w[2 * kh:, c:c + 128] for c in (c0, c1)], axis=1))
            return st["r"]

        def m1():
            st[1] = dot(A(0, 0), B(0, c0))
            return st[1]

        def m2():
            st[11] = R(0, 0, st[1] + dot(A(0, 1), B(1, c0)))
            return st[11]

        def m6():
            st[2] = st[1] + dot(s(1), T(1))
            return st[2]

        def m7():
            st[3] = st[2] + dot(s(2), T(2))
            return st[3]

        def m4():
            y = R(1, 0, st[3] - dot(A(1, 1), T(3)))
            fin(c0, jnp.concatenate([st[11], y], axis=0))
            return y

        def m5():
            y = dot(s(0), T(0))
            st[22], st[4] = R(1, 1, st[3] + y), st[2] + y
            return st[4]

        def m3():
            y = R(0, 1, st[4] + dot(s(3), B(1, c1)))
            fin(c1, jnp.concatenate([y, st[22]], axis=0))
            return y
        return [(128, rem)] * (w.shape[0] > 2 * kh) + [(kh // 4, m) for m in (m1, m2, m6, m7, m4, m5, m3)]

    def norm(t, slot):
        y = _ln(x_s[rows(jnp.minimum(t, STEPS - 1)), :].astype(f32))
        _Packed(xn_s.at[t % 2 + slot])[:, :] = y.astype(bf16)
        if slot == 0:
            for n, v in enumerate(_sums(y, 256)):
                xs_s[t % 2, n] = pltpu.bitcast(v, i32)

    def qkv_items(t, slot):
        vts = {}
        xn = lambda: _Packed(xn_s.at[t % 2 + slot])
        xs = lambda n: pltpu.bitcast(xs_s[t % 2, n], bf16)
        lo = iota((TB // 2, 128), 1) < 64
        half = pl.ds(pl.multiple_of(t * (TB // 2), TB // 2), TB // 2)

        def slab(dst, scale):
            ys = {}

            def fin(c, y):
                j = c % D // 128
                ys[j] = y = pltpu.bitcast((y * scale if scale else y).astype(bf16), i32)
                if j != 2:
                    later.append(lambda: dst.__setitem__(((0, 2, None, 5, 7)[j], half), y))
                for jj in (j, j + 1):
                    if jj in ys and jj - 1 in ys:
                        m = jnp.where(lo, ys[jj], ys[jj - 1])
                        later.append(lambda m=m, jj=jj: dst.__setitem__(((None, 1, 3, 4, 6)[jj], half), m))
            return fin

        def vfin(c, y):
            j = c % D // 128
            vts[j] = pltpu.bitcast(pltpu.bitcast(_ilv(y, True), bf16).T, i32)
            sub = iota((8, TB), 0)
            for h in range(H):
                r0 = DH * h // 16 * 8
                need = (r0 // 64, (r0 + 8) // 64)
                if j not in need or need[0] not in vts or need[1] not in vts:
                    continue
                a, b = (vts[r // 64][r % 64:r % 64 + 8] for r in (r0, r0 + 8))
                if h % 4 < 2:
                    b = jnp.where(sub >= 4, ONES, b)
                else:
                    a = jnp.where(sub < 4, ONES, a)
                w = jnp.concatenate([a, b], axis=0)
                for bb in range(NB):
                    later.append(lambda w=w, h=h, bb=bb:
                                 vt_s.__setitem__((t * NB + bb, h), w[:, 128 * bb:128 * (bb + 1)]))
        fins = (slab(q_s, DH ** -0.5 * LOG2E), slab(k_s, None), vfin)
        if slot:
            return [lin(xn, wqkv, D * n, D, fins[n], 512 if n else QA) for n in range(3)]
        fin = lambda c, y: fins[c // D](c, y)
        return sum((pair(xn, xs, wqkv, tq, 128 * n, c0, c1, fin) for n, (c0, c1) in enumerate(QP)), []) \
            + lin(xn, wqkv, 2 * D + 512, 128, fin)

    def mlp_items(t, gate=None, hoist=0, mid=None):
        hs, gs, ss, st = [], {}, [], {}

        def once(key, fn):
            if key not in st:
                st[key] = fn()
            return st[key]

        def f_o(c, y):
            hs.append(x_s[rows(t), c:c + 128].astype(f32) + y)

        def f_up(c, y):
            gs[c] = jax.nn.gelu(y + b1_s[c:c + 128].astype(f32).reshape(1, 128), approximate=True)
            if c >= F // 2:
                ss.append(_sums(jnp.concatenate([gs[c - F // 2], gs[c]], axis=1), 128))

        def f_dn(c, y):
            y = y + b2_s[c:c + 128].astype(f32).reshape(1, 128)
            out_s[rows(t), c:c + 128] = (hs[c // 128] + y).astype(bf16)
        o = pltpu.bitcast(o_s[...], bf16)
        hf = lambda: once("hf", lambda: _ln(jnp.concatenate(hs, axis=1), gate))
        hn = lambda: once("hn", lambda: hf().astype(bf16))
        h4 = lambda n: once("h4", lambda: _sums(hf(), 256))[n]
        u = lambda: once("u", lambda: jnp.concatenate([gs[c].astype(bf16) for c in sorted(gs)], axis=1))
        u4 = lambda n: once(("u4", n), lambda: jnp.concatenate([v[n] for v in ss], axis=1))
        up = sum((pair(hn, h4, w1, t1, c, c, c + F // 2, f_up) for c in range(0, F // 2, 128)), [])
        dn = [lin(u, w2, 512, 128, f_dn)] + [pair(u, u4, w2, t2, c, c, c + 256, f_dn) for c in (0, 128)]
        dn = dn[1] + dn[2] + [(0, mid)] + dn[0] if mid else dn[0] + dn[1] + dn[2]
        if not hoist:
            return lin(lambda: o, wo, 0, D, f_o), up + dn
        top = {}
        m0 = lin(lambda: o[:128], wo, 0, D, top.__setitem__)
        m0 += lin(lambda: o[128:], wo, 0, D, lambda c, y: f_o(c, jnp.concatenate([top[c], y], axis=0)))
        early = [8 * n + 1 for n in range(hoist)]
        up = [up[n] for n in early] + [v for n, v in enumerate(up) if n not in early]
        return [(w // 2, it) for w, it in m0], up + dn

    class Unit:
        def __init__(self, n, first, ot):
            self.g, self.b, self.ot = n % NG, n // NG, ot
            self.nprev = min(self.b, 2) if first else 2
            self.f, self.p = (f0, f1)[n % 2], (p0, p1)[n % 2]
            self.zs, self.zl = (0, 0) if first else (i // 1024, i // 2048)
            self.mx, self.blk = [None] * 4, i * NB + self.b

        def qk(self, j):
            g = self.g
            qb = q_s[g, pl.ds(pl.multiple_of(self.blk * 64 + 16 * j, 16), 16), :].reshape(2, 8, 128)
            parts = []
            for grp in range(4):
                own = ((iota((8, 128), 1) - DH * (4 * g + (j - grp) % 4)) & 127) < DH
                parts.append((qb & jnp.where(own, -1, 0)[None]).reshape(16, 128))
            qm = pltpu.bitcast(jnp.concatenate(parts, axis=0), bf16)
            ts = max(0, 256 - 128 * self.nprev - 32 * j)
            k0 = pl.multiple_of(self.blk * 64 - 128 + 16 * j + ts // 2, 16)
            kk = pltpu.bitcast(k_s[g, pl.ds(k0, 144 - ts // 2), :], bf16)
            s = jax.lax.dot_general(kk, qm, (((1,), (1,)), ((), ())), preferred_element_type=f32)
            mx = jnp.where(iota((32, 128), 0) > (iota((32, 128), 1) & 31),
                           s[:32] if ts == 0 else MASKED, s[256 - ts:])
            self.f[self.zs, j, 32 * j:32 * j + 32] = mx
            for t in range(32, 256, 32):
                r = (32 * j + t) % 256
                if t >= ts:
                    v = s[t - ts:t - ts + 32]
                    mx = jnp.maximum(mx, v)
                    self.f[self.zs, j, r:r + 32] = v
                elif r < 128:
                    self.f[self.zs, j, r:r + 32] = jnp.full((32, 128), MASKED, f32)
            self.mx[j] = jnp.broadcast_to(jnp.max(mx, axis=0, keepdims=True), (8, 128))

        def ex(self, c, nc, tick):
            n = (256 if self.nprev else 128) // nc
            mx = [m if tick is None else jnp.where(never, tick, m) for m in self.mx]
            for r in range(c * n, (c + 1) * n, 16):
                p = [_ilv(jnp.exp2((self.f[self.zl, j, r:r + 16].reshape(2, 8, 128) - mx[j][None]).reshape(16, 128)),
                          False) for j in range(4)]
                for hh, v in enumerate(_merge(p)):
                    self.p[self.zs, hh, r // 2:r // 2 + 8] = v

        def pv(self, hh):
            h = 4 * self.g + hh
            mm = lambda back, p: dot(pltpu.bitcast(vt_s[self.blk - back, h], bf16), pltpu.bitcast(p, bf16))
            pf = self.p[self.zl, hh, 0:64]
            if self.nprev == 2:
                pa = pf & tri_s[hh]
                pf = pf ^ pa
            o = mm(0, pf)
            if self.nprev >= 1:
                o += mm(1, self.p[self.zl, hh, 64:128])
            if self.nprev == 2:
                o += mm(2, pa)
            l, o = (o[24:], o[:24]) if hh < 2 else (o[:8], o[8:])
            o = (o.reshape(3, 8, 128) * (1.0 / l)[None]).reshape(24, 128)
            if hh:
                o = pltpu.roll(o, 32 * hh, 1)
            self.ot.append(o[4 * (hh % 2):4 * (hh % 2) + DH])
            c = (h + 1) * DH // 128 * 128
            if c > h * DH // 128 * 128:
                o = jnp.concatenate(self.ot, axis=0)[c - 128:c]
                o_s[64 * self.b:64 * self.b + 64, c - 128:c] = pltpu.bitcast(o.T.astype(bf16), i32)

    def attend(first, dense, head, tail, tie):
        ots = [[] for _ in range(NB)]
        n, nc = NB * NG, (8 if first else 16)
        us = [Unit(t, first, ots[t // NG]) for t in range(n)]
        tot, done = sum(w for w, _ in dense), 0

        def advance(upto):
            nonlocal done
            out = []
            while dense and done + dense[0][0] // 2 <= upto:
                w, it = dense.pop(0)
                done += w
                y = it()
                if w:
                    out.append((w, y))
                    seen.append(y)
            return out
        advance(head)
        for t in range(n + 2):
            if t < n:
                for j in range(4):
                    us[t].qk(j)
            flush()
            if t >= 2:
                for j in range(4):
                    us[t - 2].pv(j)
            ys = advance(head + (tot - head - tail) * t // n if t <= n else tot)
            if 1 <= t <= n:
                for c in range(nc):
                    tick, pos = None, int(c * sum(w for w, _ in ys) * tie) // nc
                    for w, y in ys:
                        if pos < w:
                            r = pos * y.shape[0] // w // 8 * 8
                            tick = y[r:r + 8, :128]
                            break
                        pos -= w
                    us[t - 1].ex(c, nc, tick)
        flush()

    @pl.when(i == 0)
    def _():
        for c in cps[:7]:
            c.start()
        for hh in range(4):
            edge = iota((128, 128), 0) > ((iota((128, 128), 1) + 32 * hh) & 127)
            tri_s[hh] = _ilv(pltpu.bitcast(jnp.where(edge, -1, 0), f32), False)

        def go(items):
            last = max(n for n, (w, _) in enumerate(items) if w)
            for n, (w, it) in enumerate(items):
                defer[:] = [1] * (n == last)
                y = it()
                if w:
                    seen.append(y)
            defer.clear()
        prep_q = lambda n: sum((prep(wqkv, tq, 128 * m, *QP[m]) for m in range(len(QP)) if QP[m][1] // D == n), [])
        a, b, na = qkv_items(0, 2), qkv_items(1, 2), 1 + QA // 128
        cps[0].wait()
        norm(0, 2)
        cps[1].wait()
        go(a[0][:na])
        norm(1, 2)
        go(b[0][:na])
        cps[2].wait()
        flush()
        go(_mix(a[0][na:] + b[0][na:], prep_q(0)))
        for c in cps[7:]:
            c.start()
        cps[3].wait()
        flush()
        go(_mix(a[1], prep_q(1)))
        cps[4].wait()
        flush()
        go(_mix(a[2], prep_q(2)))
        flush()
        rest = b[1][6:] + b[2]
        rest.insert(1, (0, functools.partial(norm, 2, 0)))
        rest = rest[:2] + _mix(rest[2:], sum((prep(w1, t1, c, c, c + F // 2) for c in range(0, F // 2, 128)), []))
        attend(True, b[1][:6] + [(0, cps[5].wait), (0, cps[6].wait)] + rest, 256, 1400, 0.5)

    @pl.when(i == 1)
    def _():
        seen.clear()
        for c in cps[7:11]:
            c.wait()
        for _, it in prep(w2, t2, 0, 0, 256) + prep(w2, t2, 128, 128, 384):
            it()

    pl.when(i == 2)(cps[11].wait)
    pl.when(i >= 2)(lambda: put(i - 2, 0, D, i - 2).start())

    @pl.when((i > 0) & (i < STEPS - 1))
    def _():
        def gate(m):
            ticks = [seen[14 + 36 * (c // 2) // 16][0:8, 0:1] for c in range(TB // 8)]
            return jnp.where(iota((TB, 1), 0) < i // 4096, jnp.concatenate(ticks, axis=0), m)
        m0, m1 = mlp_items(i - 1, gate)
        norm(i + 2, 0)
        attend(False, m0 + qkv_items(i + 1, 0) + m1, 384, 768, 0.55)

    @pl.when(i == STEPS - 1)
    def _():
        seen.clear()
        attend(False, sum(mlp_items(i - 1, hoist=4), []), 1700, 576, 0.7)
        put(STEPS - 2, 0, D, STEPS - 2).start()
        last = [put(STEPS - 1, 0, 512, STEPS - 1), put(STEPS - 1, 512, D, STEPS)]
        for _, it in sum(mlp_items(i, hoist=6, mid=last[0].start), []):
            it()
        last[1].start()
        for c in [put(t, 0, D, t) for t in range(STEPS - 1)] + last:
            c.wait()


def run(A_x, A_wqkv, A_wo, B_x, B_w1, B_b1, B_w2, B_b2):
    del B_x
    hbm = pl.BlockSpec(memory_space=pl.ANY)
    words = lambda *shapes: [pltpu.VMEM(s, i32) for s in shapes]
    return pl.pallas_call(
        _kernel,
        grid=(STEPS,),
        in_specs=[hbm] * 7,
        out_specs=hbm,
        out_shape=jax.ShapeDtypeStruct((1, S, D), bf16),
        scratch_shapes=[
            pltpu.VMEM((S, D), bf16), pltpu.SemaphoreType.DMA((STEPS + 1,)),
            pltpu.VMEM((F,), bf16), pltpu.VMEM((D,), bf16), pltpu.VMEM((S, D), bf16),
            *[pltpu.VMEM(s, bf16) for s in ((D, 3 * D), (D, D), (D, F), (F, D))],
            *words((NG, S // 2, 128), (NG, S // 2, 128), (S // 128, H, 16, 128), (TB // 2, D)),
            pltpu.SemaphoreType.DMA((12,)),
            *words((4, 64, 128), (4, TB // 2, D), (2, 4, 64, 256)),
            *words((4, 128, 128 * len(QP)), (4, 128, F // 2), (4, F // 4, 256)),
            *[pltpu.VMEM((1, 4, 256, 128), f32)] * 2, *words((1, 4, 128, 128), (1, 4, 128, 128))],
        compiler_params=pltpu.CompilerParams(dimension_semantics=("arbitrary",),
                                             vmem_limit_bytes=100 * 1024 * 1024),
    )(A_x, A_wqkv, A_wo, B_w1, B_b1, B_w2, B_b2)


@jax.jit
def pallas_sequential_preLN__sliding_block__dense_activation_gelu__prompt_kernel(
        A_x, A_wqkv, A_wo, B_x, B_w1, B_b1, B_w2, B_b2):
    return run(A_x, A_wqkv, A_wo, B_x, B_w1, B_b1, B_w2, B_b2)
```

```python
import functools

import jax
import jax.numpy as jnp
import jax.experimental.pallas as pl
import jax.experimental.pallas.tpu as pltpu

S, D, F, H = 2048, 640, 1536, 32
DH = D // H
NG = H // 4
TB = 256
NB = TB // 128
STEPS = S // TB
LOG2E = 1.4426950408889634
MASKED = -1e9 * LOG2E
ONES = 0x3F803F80
QA = 256
QP = [(D * n + c, D * n + c + 128) for n in range(3) for c in (0, 256)]
bf16, f32, i32 = jnp.bfloat16, jnp.float32, jnp.int32
dot = functools.partial(jnp.dot, preferred_element_type=f32)
iota = functools.partial(jax.lax.broadcasted_iota, i32)


def _ln(x, gate=None):
    m = jnp.mean(x, axis=-1, keepdims=True)
    if gate:
        m = gate(m)
    xc = x - m
    v = jnp.mean(xc * xc, axis=-1, keepdims=True)
    return xc * jax.lax.rsqrt(v + 1e-5)


def _ilv(y, rnd):
    n, c = y.shape
    b = pltpu.bitcast(y, i32)
    if rnd:
        b = b + 0x8000
    b = b.reshape(n // 16, 2, 8, c)
    return (jax.lax.shift_right_logical(b[:, 0], 16) | (b[:, 1] & -65536)).reshape(n // 2, c)


def _mix(a, b):
    keyed = [(n / len(a), x) for n, x in enumerate(a)] + [(n / (len(b) + 1), x) for n, x in enumerate(b)]
    return [it for _, it in sorted(keyed, key=lambda q: q[0])]


def _merge(p):
    c = iota(p[0].shape, 1)
    odd, high = (c & 32) != 0, (c & 64) != 0
    u = [jnp.where(odd, p[(a + 1) % 4], p[a]) for a in range(4)]
    return [jnp.where(high, u[(a + 2) % 4], u[a]) for a in range(4)]


def _sums(y, kh):
    a11, a12, a21, a22 = y[:128, :kh], y[:128, kh:2 * kh], y[128:, :kh], y[128:, kh:2 * kh]
    s1 = a21 + a22
    s2 = s1 - a11
    return [v.astype(bf16) for v in (s1, s2, a11 - a21, a12 - s2)]


class _Packed:
    def __init__(self, r):
        self.r, self.shape = r, r.shape[:-2] + (r.shape[-2] * 2, r.shape[-1])

    def _ix(self, ix):
        *a, k, c = ix
        return (*a, slice((k.start or 0) // 2, (k.stop or self.shape[-2]) // 2), c)

    def __getitem__(self, ix):
        return pltpu.bitcast(self.r[self._ix(ix)], bf16)

    def __setitem__(self, ix, v):
        self.r[self._ix(ix)] = pltpu.bitcast(v, i32)


def _kernel(x_h, wqkv_h, wo_h, w1_h, b1_h, w2_h, b2_h, out_h, out_s, osem, b1_s, b2_s, x_s, wqkv, wo, w1, w2,
            q_s, k_s, vt_s, o_s, sem, tri_s, xn_s, xs_s, tq, t1, t2, f0, f1, p0, p1):
    i = pl.program_id(0)
    moves = [(x_h.at[0, 0:2 * TB], x_s.at[0:2 * TB])]
    moves += [(wqkv_h.at[:, c:e], wqkv.at[:, c:e]) for c, e in ((0, QA), (QA, D), (D, 2 * D), (2 * D, 3 * D))]
    moves += [(x_h.at[0, 2 * TB:4 * TB], x_s.at[2 * TB:4 * TB]), (w1_h, w1), (w2_h, w2),
              (wo_h, wo), (b1_h, b1_s), (b2_h, b2_s), (x_h.at[0, 4 * TB:S], x_s.at[4 * TB:S])]
    cps = [pltpu.make_async_copy(s, d, sem.at[n]) for n, (s, d) in enumerate(moves)]
    tq, t1, t2 = map(_Packed, (tq, t1, t2))

    never = iota((8, 128), 1) < i // 4096
    seen, used, later, defer = [], {}, [], []

    def rows(t):
        return pl.ds(pl.multiple_of(t * TB, TB), TB)

    def flush():
        for fn in later:
            fn()
        later.clear()

    def put(t, c, e, n):
        r = rows(t) if isinstance(t, jax.Array) else pl.ds(t * TB, TB)
        return pltpu.make_async_copy(out_s.at[r, c:e], out_h.at[0, r, c:e], osem.at[n])

    def lin(a, w, c0, n, fin, first=512):
        items, st, kk = [], {}, w.shape[0]
        cuts = [0] + list(range(first, n, 512)) + [n]
        for c, e in zip(cuts, cuts[1:]):
            if kk % 512:
                def rem(c=c, e=e):
                    st[c] = dot(a()[:, 512:], w[512:, c0 + c:c0 + e])
                    return st[c]
                items.append(((e - c) // 2, rem))
            for cc in range(c, e, 128):
                for k in range(0, kk - 511, 512):
                    def main(c=c, cc=cc, k=k):
                        y = dot(a()[:, k:k + 512], w[k:k + 512, c0 + cc:c0 + cc + 128])
                        if k:
                            y = y + st["acc"]
                        elif kk % 512:
                            y = y + st[c][:, cc - c:cc - c + 128]
                        st["acc"] = y
                        if k + 1024 > kk:
                            later.append(lambda: fin(c0 + cc, y)) if defer else fin(c0 + cc, y)
                        return y
                    items.append((256, main))
        return items

    def prep(w, t, tc, c0, c1):
        kh, items = t.shape[1], []
        for k in range(0, kh, 128):
            def it(k=k):
                b11, b12, b21, b22 = (w[r:r + 128, c:c + 128].astype(f32) for r in (k, k + kh) for c in (c0, c1))
                if seen:
                    r = used.get(len(seen), 0) * 64 % seen[-1].shape[0]
                    used[len(seen)] = used.get(len(seen), 0) + 1
                    b12 = jnp.where(never[None], seen[-1][r:r + 8, :128][None],
                                    b12.reshape(16, 8, 128)).reshape(128, 128)
                u1 = b12 - b11
                u2 = b22 - u1
                for n, v in enumerate((u1, u2, b22 - b12, u2 - b21)):
                    t[n, k:k + 128, tc:tc + 128] = v.astype(bf16)
            items.append((0, it))
        return items

    def pair(a, s, w, t, tc, c0, c1, fin):
        kh, st = t.shape[1], {}
        A = lambda r, k: a()[128 * r:128 * r + 128, kh * k:kh * k + kh]
        B = lambda k, c: w[kh * k:kh * k + kh, c:c + 128]
        T = lambda n: t[n, :, tc:tc + 128]
        R = lambda r, c, y: y + st["r"][128 * r:128 * r + 128, 128 * c:128 * c + 128] if "r" in st else y

        def rem():
            st["r"] = dot(a()[:, 2 * kh:], jnp.concatenate([w[2 * kh:, c:c + 128] for c in (c0, c1)], axis=1))
            return st["r"]

        def m1():
            st[1] = dot(A(0, 0), B(0, c0))
            return st[1]

        def m2():
            st[11] = R(0, 0, st[1] + dot(A(0, 1), B(1, c0)))
            return st[11]

        def m6():
            st[2] = st[1] + dot(s(1), T(1))
            return st[2]

        def m7():
            st[3] = st[2] + dot(s(2), T(2))
            return st[3]

        def m4():
            y = R(1, 0, st[3] - dot(A(1, 1), T(3)))
            fin(c0, jnp.concatenate([st[11], y], axis=0))
            return y

        def m5():
            y = dot(s(0), T(0))
            st[22], st[4] = R(1, 1, st[3] + y), st[2] + y
            return st[4]

        def m3():
            y = R(0, 1, st[4] + dot(s(3), B(1, c1)))
            fin(c1, jnp.concatenate([y, st[22]], axis=0))
            return y
        return [(128, rem)] * (w.shape[0] > 2 * kh) + [(kh // 4, m) for m in (m1, m2, m6, m7, m4, m5, m3)]

    def norm(t, slot):
        y = _ln(x_s[rows(jnp.minimum(t, STEPS - 1)), :].astype(f32))
        _Packed(xn_s.at[t % 2 + slot])[:, :] = y.astype(bf16)
        if slot == 0:
            for n, v in enumerate(_sums(y, 256)):
                xs_s[t % 2, n] = pltpu.bitcast(v, i32)

    def qkv_items(t, slot):
        vts = {}
        xn = lambda: _Packed(xn_s.at[t % 2 + slot])
        xs = lambda n: pltpu.bitcast(xs_s[t % 2, n], bf16)
        lo = iota((TB // 2, 128), 1) < 64
        half = pl.ds(pl.multiple_of(t * (TB // 2), TB // 2), TB // 2)

        def slab(dst, scale):
            ys = {}

            def fin(c, y):
                j = c % D // 128
                ys[j] = y = pltpu.bitcast((y * scale if scale else y).astype(bf16), i32)
                if j != 2:
                    later.append(lambda: dst.__setitem__(((0, 2, None, 5, 7)[j], half), y))
                for jj in (j, j + 1):
                    if jj in ys and jj - 1 in ys:
                        m = jnp.where(lo, ys[jj], ys[jj - 1])
                        later.append(lambda m=m, jj=jj: dst.__setitem__(((None, 1, 3, 4, 6)[jj], half), m))
            return fin

        def vfin(c, y):
            j = c % D // 128
            vts[j] = pltpu.bitcast(pltpu.bitcast(_ilv(y, True), bf16).T, i32)
            sub = iota((8, TB), 0)
            for h in range(H):
                r0 = DH * h // 16 * 8
                need = (r0 // 64, (r0 + 8) // 64)
                if j not in need or need[0] not in vts or need[1] not in vts:
                    continue
                a, b = (vts[r // 64][r % 64:r % 64 + 8] for r in (r0, r0 + 8))
                if h % 4 < 2:
                    b = jnp.where(sub >= 4, ONES, b)
                else:
                    a = jnp.where(sub < 4, ONES, a)
                w = jnp.concatenate([a, b], axis=0)
                for bb in range(NB):
                    later.append(lambda w=w, h=h, bb=bb:
                                 vt_s.__setitem__((t * NB + bb, h), w[:, 128 * bb:128 * (bb + 1)]))
        fins = (slab(q_s, DH ** -0.5 * LOG2E), slab(k_s, None), vfin)
        if slot:
            return [lin(xn, wqkv, D * n, D, fins[n], 512 if n else QA) for n in range(3)]
        fin = lambda c, y: fins[c // D](c, y)
        return sum((pair(xn, xs, wqkv, tq, 128 * n, c0, c1, fin)
                    + (lin(xn, wqkv, c1 + 128, 128, fin) if n % 2 else []) for n, (c0, c1) in enumerate(QP)), [])

    def mlp_items(t, gate=None, hoist=0, mid=None):
        hs, gs, ss, st = [], {}, [], {}

        def once(key, fn):
            if key not in st:
                st[key] = fn()
            return st[key]

        def f_o(c, y):
            hs.append(x_s[rows(t), c:c + 128].astype(f32) + y)

        def f_up(c, y):
            gs[c] = jax.nn.gelu(y + b1_s[c:c + 128].astype(f32).reshape(1, 128), approximate=True)
            if c >= F // 2:
                ss.append(_sums(jnp.concatenate([gs[c - F // 2], gs[c]], axis=1), 128))

        def f_dn(c, y):
            y = y + b2_s[c:c + 128].astype(f32).reshape(1, 128)
            out_s[rows(t), c:c + 128] = (hs[c // 128] + y).astype(bf16)
        o = pltpu.bitcast(o_s[...], bf16)
        hf = lambda: once("hf", lambda: _ln(jnp.concatenate(hs, axis=1), gate))
        hn = lambda: once("hn", lambda: hf().astype(bf16))
        h4 = lambda n: once("h4", lambda: _sums(hf(), 256))[n]
        u = lambda: once("u", lambda: jnp.concatenate([gs[c].astype(bf16) for c in sorted(gs)], axis=1))
        u4 = lambda n: once(("u4", n), lambda: jnp.concatenate([v[n] for v in ss], axis=1))
        up = sum((pair(hn, h4, w1, t1, c, c, c + F // 2, f_up) for c in range(0, F // 2, 128)), [])
        dn = [lin(u, w2, 512, 128, f_dn)] + [pair(u, u4, w2, t2, c, c, c + 256, f_dn) for c in (0, 128)]
        dn = dn[1] + dn[2] + [(0, mid)] + dn[0] if mid else dn[0] + dn[1] + dn[2]
        if not hoist:
            return lin(lambda: o, wo, 0, D, f_o), up + dn
        top = {}
        m0 = lin(lambda: o[:128], wo, 0, D, top.__setitem__)
        m0 += lin(lambda: o[128:], wo, 0, D, lambda c, y: f_o(c, jnp.concatenate([top[c], y], axis=0)))
        early = [8 * n + 1 for n in range(hoist)]
        up = [up[n] for n in early] + [v for n, v in enumerate(up) if n not in early]
        return [(w // 2, it) for w, it in m0], up + dn

    class Unit:
        def __init__(self, n, first, ot):
            self.g, self.b, self.ot = n % NG, n // NG, ot
            self.nprev = min(self.b, 2) if first else 2
            self.f, self.p = (f0, f1)[n % 2], (p0, p1)[n % 2]
            self.zs, self.zl = (0, 0) if first else (i // 1024, i // 2048)
            self.mx, self.blk = [None] * 4, i * NB + self.b

        def qk(self, j):
            g = self.g
            qb = q_s[g, pl.ds(pl.multiple_of(self.blk * 64 + 16 * j, 16), 16), :].reshape(2, 8, 128)
            parts = []
            for grp in range(4):
                own = ((iota((8, 128), 1) - DH * (4 * g + (j - grp) % 4)) & 127) < DH
                parts.append((qb & jnp.where(own, -1, 0)[None]).reshape(16, 128))
            qm = pltpu.bitcast(jnp.concatenate(parts, axis=0), bf16)
            ts = max(0, 256 - 128 * self.nprev - 32 * j)
            k0 = pl.multiple_of(self.blk * 64 - 128 + 16 * j + ts // 2, 16)
            kk = pltpu.bitcast(k_s[g, pl.ds(k0, 144 - ts // 2), :], bf16)
            s = jax.lax.dot_general(kk, qm, (((1,), (1,)), ((), ())), preferred_element_type=f32)
            mx = jnp.where(iota((32, 128), 0) > (iota((32, 128), 1) & 31),
                           s[:32] if ts == 0 else MASKED, s[256 - ts:])
            self.f[self.zs, j, 32 * j:32 * j + 32] = mx
            for t in range(32, 256, 32):
                r = (32 * j + t) % 256
                if t >= ts:
                    v = s[t - ts:t - ts + 32]
                    mx = jnp.maximum(mx, v)
                    self.f[self.zs, j, r:r + 32] = v
                elif r < 128:
                    self.f[self.zs, j, r:r + 32] = jnp.full((32, 128), MASKED, f32)
            self.mx[j] = jnp.broadcast_to(jnp.max(mx, axis=0, keepdims=True), (8, 128))

        def ex(self, c, nc, tick):
            n = (256 if self.nprev else 128) // nc
            mx = [m if tick is None else jnp.where(never, tick, m) for m in self.mx]
            for r in range(c * n, (c + 1) * n, 16):
                p = [_ilv(jnp.exp2((self.f[self.zl, j, r:r + 16].reshape(2, 8, 128) - mx[j][None]).reshape(16, 128)),
                          False) for j in range(4)]
                for hh, v in enumerate(_merge(p)):
                    self.p[self.zs, hh, r // 2:r // 2 + 8] = v

        def pv(self, hh):
            h = 4 * self.g + hh
            mm = lambda back, p: dot(pltpu.bitcast(vt_s[self.blk - back, h], bf16), pltpu.bitcast(p, bf16))
            pf = self.p[self.zl, hh, 0:64]
            if self.nprev == 2:
                pa = pf & tri_s[hh]
                pf = pf ^ pa
            o = mm(0, pf)
            if self.nprev >= 1:
                o += mm(1, self.p[self.zl, hh, 64:128])
            if self.nprev == 2:
                o += mm(2, pa)
            l, o = (o[24:], o[:24]) if hh < 2 else (o[:8], o[8:])
            o = (o.reshape(3, 8, 128) * (1.0 / l)[None]).reshape(24, 128)
            if hh:
                o = pltpu.roll(o, 32 * hh, 1)
            self.ot.append(o[4 * (hh % 2):4 * (hh % 2) + DH])
            c = (h + 1) * DH // 128 * 128
            if c > h * DH // 128 * 128:
                o = jnp.concatenate(self.ot, axis=0)[c - 128:c]
                o_s[64 * self.b:64 * self.b + 64, c - 128:c] = pltpu.bitcast(o.T.astype(bf16), i32)

    def attend(first, dense, head, tail, tie):
        ots = [[] for _ in range(NB)]
        n, nc = NB * NG, (8 if first else 16)
        us = [Unit(t, first, ots[t // NG]) for t in range(n)]
        tot, done = sum(w for w, _ in dense), 0

        def advance(upto):
            nonlocal done
            out = []
            while dense and done + dense[0][0] // 2 <= upto:
                w, it = dense.pop(0)
                done += w
                y = it()
                if w:
                    out.append((w, y))
                    seen.append(y)
            return out
        advance(head)
        for t in range(n + 2):
            if t < n:
                for j in range(4):
                    us[t].qk(j)
            flush()
            if t >= 2:
                for j in range(4):
                    us[t - 2].pv(j)
            ys = advance(head + (tot - head - tail) * t // n if t <= n else tot)
            if 1 <= t <= n:
                for c in range(nc):
                    tick, pos = None, int(c * sum(w for w, _ in ys) * tie) // nc
                    for w, y in ys:
                        if pos < w:
                            r = pos * y.shape[0] // w // 8 * 8
                            tick = y[r:r + 8, :128]
                            break
                        pos -= w
                    us[t - 1].ex(c, nc, tick)
        flush()

    @pl.when(i == 0)
    def _():
        for c in cps[:7]:
            c.start()
        for hh in range(4):
            edge = iota((128, 128), 0) > ((iota((128, 128), 1) + 32 * hh) & 127)
            tri_s[hh] = _ilv(pltpu.bitcast(jnp.where(edge, -1, 0), f32), False)

        def go(items):
            last = max(n for n, (w, _) in enumerate(items) if w)
            for n, (w, it) in enumerate(items):
                defer[:] = [1] * (n == last)
                y = it()
                if w:
                    seen.append(y)
            defer.clear()
        prep_q = lambda n: sum((prep(wqkv, tq, 128 * m, *QP[m]) for m in range(len(QP)) if QP[m][1] // D == n), [])
        a, b, na = qkv_items(0, 2), qkv_items(1, 2), 1 + QA // 128
        cps[0].wait()
        norm(0, 2)
        cps[1].wait()
        go(a[0][:na])
        norm(1, 2)
        go(b[0][:na])
        cps[2].wait()
        flush()
        go(_mix(a[0][na:] + b[0][na:], prep_q(0)))
        for c in cps[7:]:
            c.start()
        cps[3].wait()
        flush()
        go(_mix(a[1], prep_q(1)))
        cps[4].wait()
        flush()
        go(_mix(a[2], prep_q(2)))
        flush()
        rest = b[1][6:] + b[2]
        rest.insert(1, (0, functools.partial(norm, 2, 0)))
        rest = rest[:2] + _mix(rest[2:], sum((prep(w1, t1, c, c, c + F // 2) for c in range(0, F // 2, 128)), []))
        attend(True, b[1][:6] + [(0, cps[5].wait), (0, cps[6].wait)] + rest, 256, 1400, 0.5)

    @pl.when(i == 1)
    def _():
        seen.clear()
        for c in cps[7:11]:
            c.wait()
        for _, it in prep(w2, t2, 0, 0, 256) + prep(w2, t2, 128, 128, 384):
            it()

    pl.when(i == 2)(cps[11].wait)
    pl.when(i >= 2)(lambda: put(i - 2, 0, D, i - 2).start())

    @pl.when((i > 0) & (i < STEPS - 1))
    def _():
        def gate(m):
            ticks = [seen[12 + 26 * (c // 2) // 16][0:8, 0:1] for c in range(TB // 8)]
            return jnp.where(iota((TB, 1), 0) < i // 4096, jnp.concatenate(ticks, axis=0), m)
        m0, m1 = mlp_items(i - 1, gate)
        norm(i + 2, 0)
        attend(False, m0 + qkv_items(i + 1, 0) + m1, 384, 832, 0.5)

    @pl.when(i == STEPS - 1)
    def _():
        seen.clear()
        attend(False, sum(mlp_items(i - 1, hoist=3), []), 1750, 640, 0.7)
        put(STEPS - 2, 0, D, STEPS - 2).start()
        last = [put(STEPS - 1, 0, 512, STEPS - 1), put(STEPS - 1, 512, D, STEPS)]
        for _, it in sum(mlp_items(i, hoist=6, mid=last[0].start), []):
            it()
        last[1].start()
        for c in [put(t, 0, D, t) for t in range(STEPS - 1)] + last:
            c.wait()


def run(A_x, A_wqkv, A_wo, B_x, B_w1, B_b1, B_w2, B_b2):
    del B_x
    hbm = pl.BlockSpec(memory_space=pl.ANY)
    words = lambda *shapes: [pltpu.VMEM(s, i32) for s in shapes]
    return pl.pallas_call(
        _kernel,
        grid=(STEPS,),
        in_specs=[hbm] * 7,
        out_specs=hbm,
        out_shape=jax.ShapeDtypeStruct((1, S, D), bf16),
        scratch_shapes=[
            pltpu.VMEM((S, D), bf16), pltpu.SemaphoreType.DMA((STEPS + 1,)),
            pltpu.VMEM((F,), bf16), pltpu.VMEM((D,), bf16), pltpu.VMEM((S, D), bf16),
            *[pltpu.VMEM(s, bf16) for s in ((D, 3 * D), (D, D), (D, F), (F, D))],
            *words((NG, S // 2, 128), (NG, S // 2, 128), (S // 128, H, 16, 128), (TB // 2, D)),
            pltpu.SemaphoreType.DMA((12,)),
            *words((4, 64, 128), (4, TB // 2, D), (2, 4, 64, 256)),
            *words((4, 128, 128 * len(QP)), (4, 128, F // 2), (4, F // 4, 256)),
            *[pltpu.VMEM((1, 4, 256, 128), f32)] * 2, *words((1, 4, 128, 128), (1, 4, 128, 128))],
        compiler_params=pltpu.CompilerParams(dimension_semantics=("arbitrary",),
                                             vmem_limit_bytes=100 * 1024 * 1024),
    )(A_x, A_wqkv, A_wo, B_w1, B_b1, B_w2, B_b2)


@jax.jit
def pallas_sequential_preLN__sliding_block__dense_activation_gelu__prompt_kernel(
        A_x, A_wqkv, A_wo, B_x, B_w1, B_b1, B_w2, B_b2):
    return run(A_x, A_wqkv, A_wo, B_x, B_w1, B_b1, B_w2, B_b2)
```
